```python
import os as _os
_os.environ.setdefault("JAX_PLATFORMS", "cpu")
import jax
import jax.numpy as jnp

def _softmax(x, axis=-1):
    return jax.nn.softmax(x, axis=axis)
def _gelu(x):
    return jax.nn.gelu(x, approximate=True)
def _silu(x):
    return jax.nn.silu(x)
def _sigmoid(x):
    return jax.nn.sigmoid(x)
def _layernorm(x, axis=-1, eps=1e-5):
    m = jnp.mean(x, axis=axis, keepdims=True)
    v = jnp.var(x, axis=axis, keepdims=True)
    return (x - m) / jnp.sqrt(v + eps)
def _scatter_add(tgt, idx, src, axis=0):
    return tgt.at[idx].add(src)
def _segment_sum(src, seg, n):
    return jax.ops.segment_sum(src, seg, n)
class _Rng:
    def __init__(self, key):
        self._k = key
    def _next(self):
        self._k, sub = jax.random.split(self._k)
        return sub
    def normal(self, shape):
        return jax.random.normal(self._next(), shape, dtype=jnp.bfloat16)
    def randint(self, lo, hi, shape):
        return jax.random.randint(self._next(), shape, lo, hi, dtype=jnp.int32)
    def uniform(self, shape, lo=0.0, hi=1.0):
        return jax.random.uniform(self._next(), shape, jnp.bfloat16, lo, hi)
    def permutation(self, n):
        return jax.random.permutation(self._next(), n)


kernel_name = 'concat_heads__linear_attn_block__sliding_local_dilated__prompt'

def setup_inputs():
    _rng = _Rng(jax.random.key(int.from_bytes(__import__("os").urandom(4), "little")))
    _w = (lambda a: (lambda t: t.astype(jnp.bfloat16) if jnp.issubdtype(t.dtype, jnp.floating) else t)(jnp.asarray(a)))
    def _A_setup():
        B, S, D = 1, 2048, 576
        return {
            "x": _w((lambda *s: _rng.normal(s) * 0.05)(B, S, D)),
            "wqkv": _w((lambda *s: _rng.normal(s) * 1.6)(D, 3 * D)),
            "wo": _w((lambda *s: _rng.normal(s) * 0.4)(D, D)),
        }
    _A_in = _A_setup()

    def _B_setup():
        B, S, D = 1, 2048, 576
        return {
            "x": _w((lambda *s: _rng.normal(s) * 0.2)(B, S, D)),
            "wqkv": _w((lambda *s: _rng.normal(s) * 0.2)(D, 3 * D)),
            "wo": _w((lambda *s: _rng.normal(s) * 0.05)(D, D)),
        }
    _B_in = _B_setup()

    return {
        "A_x": _A_in["x"],
        "A_wqkv": _A_in["wqkv"],
        "A_wo": _A_in["wo"],
        "B_x": _B_in["x"],
        "B_wqkv": _B_in["wqkv"],
        "B_wo": _B_in["wo"],
    }

def reference(A_x, A_wqkv, A_wo, B_x, B_wqkv, B_wo):
    def _A_ref(x, wqkv, wo):
        B, S, D = x.shape
        H = 32; Dh = D // H
        qkv = (lambda x, *d: x.transpose(*d))((x @ wqkv).reshape(B, S, 3, H, Dh), 2, 0, 3, 1, 4)
        q, k, v = qkv[0], qkv[1], qkv[2]
        phi = lambda t: jnp.where(t > 0, t + 1, jnp.exp(t)) + 1e-6
        pq, pk = phi(q), phi(k)
        kv = jnp.einsum("bhsd,bhse->bhde", pk, v)
        z = jnp.einsum("bhsd->bhd", pk)
        num = jnp.einsum("bhqd,bhde->bhqe", pq, kv)
        den = jnp.einsum("bhqd,bhd->bhq", pq, z)[..., None] + 1e-6
        o = num / den
        return (lambda x, *d: x.transpose(*d))(o, 0, 2, 1, 3).reshape(B, S, D) @ wo

    def _B_ref(x, wqkv, wo):
        B, S, D = x.shape
        H = 32; Dh = D // H
        W, dil = 8, 2
        qkv = (lambda x, *d: x.transpose(*d))((x @ wqkv).reshape(B, S, 3, H, Dh), 2, 0, 3, 1, 4)
        q, k, v = qkv[0], qkv[1], qkv[2]
        scale = Dh ** -0.5
        pos = jnp.arange(S)
        off = jnp.arange(W) * dil
        idx = pos[:, None] - off[None, :]
        mask = idx >= 0
        idx_c = jnp.where(mask, idx, 0).reshape(-1)
        kg = k[:, :, idx_c, :].reshape(B, H, S, W, Dh)
        vg = v[:, :, idx_c, :].reshape(B, H, S, W, Dh)
        logits = jnp.einsum("bhsd,bhswd->bhsw", q, kg) * scale
        logits = jnp.where(mask[None, None, :, :], logits, -1e9)
        attn = _softmax(logits, axis=-1)
        o = jnp.einsum("bhsw,bhswd->bhsd", attn, vg)
        return (lambda x, *d: x.transpose(*d))(o, 0, 2, 1, 3).reshape(B, S, D) @ wo

    a = _A_ref(A_x, A_wqkv, A_wo)
    b = _B_ref(B_x, B_wqkv, B_wo)
    return jnp.concatenate([a, b], axis=-1)
```

```python
import functools
import math

import jax
import jax.numpy as jnp
from jax import lax
import jax.experimental.pallas as pl
import jax.experimental.pallas.tpu as pltpu

S = 2048
D = 576
H = 32
DH = 18
KP = 640
BLK = 512
NB = S // BLK
HALO = 16
WIN = 8
F32 = jnp.float32
BF16 = jnp.bfloat16
LOG2E = math.log2(math.e)
CSC = (DH ** -0.5) * LOG2E
NEG = -1e9 * LOG2E
ROWS = [(0, 144), (112, 272), (240, 400), (368, 528), (496, 576)]


def _phi(t):
    return jnp.where(t > 0, t + 1.0, jnp.exp(t)) + 1e-6


def _dot(a, b):
    return jnp.dot(a, b, preferred_element_type=F32)


def _dot_nt(a, b):
    return lax.dot_general(a, b, (((1,), (1,)), ((), ())), preferred_element_type=F32)


def _ktile(w_ref, c, col0, ncol):
    if c < 4:
        return w_ref[pl.ds(128 * c, 128), pl.ds(col0, ncol)]
    blk = w_ref[pl.ds(512, 64), pl.ds(col0, ncol)]
    return jnp.concatenate([blk, jnp.zeros_like(blk)], axis=0)


def _kernel(xa_hbm, wa_hbm, woa_hbm, xb_hbm, wb_hbm, wob_hbm, out_hbm,
            xa, xb, wa, wb, woa, wob,
            wt32, wqkT, wbT, woT, mT, pq, T, zb, att, oT, scT, outbuf,
            sem_in, sem_out):
    def w_copy(name):
        if name == 'wa_qk':
            return pltpu.make_async_copy(wa_hbm.at[:, pl.ds(0, 1152)], wa.at[:, pl.ds(0, 1152)], sem_in.at[0])
        if name == 'wb':
            return pltpu.make_async_copy(wb_hbm, wb, sem_in.at[5])
        if name == 'wa_v':
            return pltpu.make_async_copy(wa_hbm.at[:, pl.ds(1152, 576)], wa.at[:, pl.ds(1152, 576)], sem_in.at[6])
        if name == 'woa':
            return pltpu.make_async_copy(woa_hbm, woa, sem_in.at[7])
        return pltpu.make_async_copy(wob_hbm, wob, sem_in.at[8])

    def xa_copy(i):
        return pltpu.make_async_copy(
            xa_hbm.at[:, pl.ds(i * BLK, BLK)], xa.at[pl.ds(0, D), pl.ds(i * BLK, BLK)], sem_in.at[1 + i])

    def xb_copy(i):
        return pltpu.make_async_copy(
            xb_hbm.at[:, pl.ds(i * BLK, BLK)], xb.at[pl.ds(0, D), pl.ds(i * BLK, BLK)], sem_in.at[9 + i])

    def out_copy(j, b):
        return pltpu.make_async_copy(
            outbuf.at[j % 2, pl.ds(b * 128, 128), :],
            out_hbm.at[pl.ds(j * BLK + b * 128, 128), :],
            sem_out.at[(j % 2) * 4 + b])

    def perm_rows(src_c, off, dst, base, c):
        for d in range(0, DH, 2):
            r0 = wt32[src_c, pl.ds(off + d, 32, stride=DH), :]
            r1 = wt32[src_c, pl.ds(off + d + 1, 32, stride=DH), :]
            dst[pl.ds(base + 32 * d, 64), pl.ds(128 * c, 128)] = jnp.concatenate([r0, r1], axis=0).astype(BF16)

    def prep_part(w_ref, col0, ncol, off, dst, base):
        for c in range(5):
            wt32[c, pl.ds(0, ncol), :] = _ktile(w_ref, c, col0, ncol).T.astype(F32)
        for c in range(5):
            perm_rows(c, off, dst, base, c)

    def phase1(i, first):
        xblk = xa[:, pl.ds(pl.multiple_of(i * BLK, BLK), BLK)]
        kT = _dot(wqkT[pl.ds(D, D), :], xblk)
        pk = _phi(kT).astype(BF16)
        for c in range(5):
            t = _dot_nt(pk, xblk[128 * c:128 * (c + 1), :])
            if first:
                T[c] = t
            else:
                T[c] += t
        qT = _dot(wqkT[pl.ds(0, D), :], xblk)
        pq[:, pl.ds(pl.multiple_of(i * BLK, BLK), BLK)] = _phi(qT)

    def b_qkv(j, first):
        slot = j % 2
        xblk = xb[:, pl.ds(pl.multiple_of(j * BLK, BLK), BLK)]
        lane = lax.broadcasted_iota(jnp.int32, (HALO, 128), 1)
        for p in range(3):
            r = _dot(wbT[pl.ds(D * p, D), :], xblk).astype(BF16)
            for d in range(DH):
                tile = jnp.concatenate(
                    [r[32 * d:32 * d + 32, 128 * b:128 * b + 128] for b in range(4)], axis=0)
                tt = tile.T.astype(F32)
                att[slot, p * DH + d, pl.ds(HALO, 128), :] = tt
                if p > 0:
                    cur = pltpu.roll(tt[128 - HALO:, :], 32, 1)
                    if first:
                        if p == 1:
                            prev = jnp.zeros((HALO, 128), F32)
                        else:
                            prev = jnp.broadcast_to(tt[0:1, :], (HALO, 128))
                    else:
                        prev = att[1 - slot, p * DH + d, pl.ds(128 + HALO, HALO), :]
                    att[slot, p * DH + d, pl.ds(0, HALO), :] = jnp.where(lane < 32, prev, cur)
                    att[slot, p * DH + d, pl.ds(128 + HALO, HALO), :] = cur

    def attention(j):
        slot = j % 2
        R = 16
        for g in range(128 // R):
            base = HALO + g * R
            ls = [None] * WIN
            for d in range(DH):
                q = att[slot, d, pl.ds(base, R), :]
                for w in range(WIN):
                    t = q * att[slot, DH + d, pl.ds(base - 2 * w, R), :]
                    ls[w] = t if ls[w] is None else ls[w] + t
            ls = [l * CSC for l in ls]
            if g == 0:
                pos = (lax.broadcasted_iota(jnp.int32, (R, 128), 0)
                       + (lax.broadcasted_iota(jnp.int32, (R, 128), 1) // 32) * 128 + j * BLK)
                ls = [ls[0]] + [jnp.where(pos >= 2 * w, ls[w], NEG) for w in range(1, WIN)]
            m = functools.reduce(jnp.maximum, ls)
            ps = [jnp.exp2(l - m) for l in ls]
            inv = 1.0 / functools.reduce(lambda a, b: a + b, ps)
            ps = [p * inv for p in ps]
            for d in range(DH):
                acc = None
                for w in range(WIN):
                    t = ps[w] * att[slot, 2 * DH + d, pl.ds(base - 2 * w, R), :]
                    acc = t if acc is None else acc + t
                att[slot, d, pl.ds(base, R), :] = acc
        for d in range(DH):
            ot = att[slot, d, pl.ds(HALO, 128), :].astype(BF16).T
            for b in range(4):
                oT[pl.ds(32 * d, 32), pl.ds(128 * b, 128)] = ot[32 * b:32 * b + 32, :]

    def a_scale(j):
        col = pl.ds(pl.multiple_of(j * BLK, BLK), BLK)
        den = None
        for d in range(DH):
            z = zb[pl.ds(32 * d, 32), :]
            z4 = jnp.concatenate([z] * 4, axis=1)
            t = pq[pl.ds(32 * d, 32), col] * z4
            den = t if den is None else den + t
        inv = 1.0 / (den + 1e-6)
        for d in range(DH):
            scT[pl.ds(32 * d, 32), :] = (pq[pl.ds(32 * d, 32), col] * inv).astype(BF16)

    def out_proj(j, wait_prev):
        slot = j % 2
        oa = _dot(mT[...], scT[...]).astype(BF16)
        ob = _dot(woT[...], oT[...]).astype(BF16)
        if wait_prev:
            for b in range(4):
                out_copy(j - 2, b).wait()
        for b in range(4):
            blk = jnp.concatenate([oa[:, 128 * b:128 * b + 128], ob[:, 128 * b:128 * b + 128]], axis=0)
            outbuf[slot, pl.ds(128 * b, 128), :] = blk.T
            out_copy(j, b).start()

    def a_small():
        for c in range(5):
            wt32[c, pl.ds(0, D), :] = jnp.zeros((D, 128), F32)
        for jt, (r0, r1) in enumerate(ROWS):
            n = r1 - r0
            w = 128 if jt < 4 else 64
            tb = jnp.concatenate([T[c, pl.ds(r0, n), :] for c in range(5)], axis=1)[:, :D].astype(BF16)
            g = _dot(tb, wa[:, pl.ds(1152 + 128 * jt, w)])
            rh = (lax.broadcasted_iota(jnp.int32, (n, w), 0) + r0) // DH
            ch = (lax.broadcasted_iota(jnp.int32, (n, w), 1) + 128 * jt) // DH
            kv = jnp.where(rh == ch, g, 0.0).astype(BF16)
            mrow = _dot(kv, woa[pl.ds(128 * jt, w), :])
            for c in range(4):
                wt32[c, pl.ds(r0, n), :] += mrow[:, 128 * c:128 * c + 128]
            wt32[4, pl.ds(r0, n), pl.ds(0, 64)] += mrow[:, 512:576]
        for c in range(5):
            nrow = 128 if c < 4 else 64
            for kt in range(5):
                ds_ = range(4 * kt, min(4 * kt + 4, DH))
                rows = [wt32[c, pl.ds(d, 32, stride=DH), :] for d in ds_]
                if kt == 4:
                    rows.append(jnp.zeros((64, 128), F32))
                tile = jnp.concatenate(rows, axis=0).astype(BF16).T
                mT[pl.ds(128 * c, nrow), pl.ds(128 * kt, 128)] = tile[:nrow, :]
        lane = lax.broadcasted_iota(jnp.int32, (32, 128), 1)
        for d in range(DH):
            t = T[4, pl.ds(d, 32, stride=DH), :]
            zb[pl.ds(32 * d, 32), :] = jnp.where(lane >= 64, t, pltpu.roll(t, 64, 1))

    def prep_wo():
        for c in range(4):
            wt32[c, pl.ds(0, D), :] = wob[:, pl.ds(128 * c, 128)].astype(F32)
        wt32[4, pl.ds(0, D), :] = jnp.concatenate(
            [wob[:, pl.ds(512, 64)].astype(F32), jnp.zeros((D, 64), F32)], axis=1)
        for c in range(5):
            nrow = 128 if c < 4 else 64
            for kt in range(5):
                ds_ = range(4 * kt, min(4 * kt + 4, DH))
                rows = [wt32[c, pl.ds(d, 32, stride=DH), :] for d in ds_]
                if kt == 4:
                    rows.append(jnp.zeros((64, 128), F32))
                tile = jnp.concatenate(rows, axis=0).astype(BF16).T
                woT[pl.ds(128 * c, nrow), pl.ds(128 * kt, 128)] = tile[:nrow, :]

    w_copy('wa_qk').start()
    for i in range(NB):
        xa_copy(i).start()
    w_copy('wb').start()
    w_copy('wa_v').start()
    w_copy('woa').start()
    w_copy('wob').start()
    for i in range(NB):
        xb_copy(i).start()
    xa[pl.ds(D, KP - D), :] = jnp.ones((KP - D, S), BF16)
    xb[pl.ds(D, KP - D), :] = jnp.zeros((KP - D, S), BF16)
    oT[pl.ds(D, KP - D), :] = jnp.zeros((KP - D, BLK), BF16)
    scT[pl.ds(D, KP - D), :] = jnp.zeros((KP - D, BLK), BF16)
    w_copy('wa_qk').wait()
    for c in range(5):
        wqkT[pl.ds(D, D), pl.ds(128 * c, 128)] = _ktile(wa, c, 512, 640).T[64:, :]
    prep_part(wa, 0, 640, 0, wqkT, 0)
    xa_copy(0).wait()
    phase1(0, True)

    xa_copy(1).wait()
    w_copy('wb').wait()
    prep_part(wb, 0, 640, 0, wbT, 0)
    phase1(1, False)

    xa_copy(2).wait()
    prep_part(wb, 512, 640, 64, wbT, D)
    phase1(2, False)

    xa_copy(3).wait()
    prep_part(wb, 1152, 576, 0, wbT, 2 * D)
    phase1(3, False)

    w_copy('wa_v').wait()
    w_copy('woa').wait()
    w_copy('wob').wait()
    xb_copy(0).wait()
    a_small()
    prep_wo()
    b_qkv(0, True)

    for j in range(1, NB):
        xb_copy(j).wait()
        b_qkv(j, False)
        attention(j - 1)
        a_scale(j - 1)
        out_proj(j - 1, j - 1 >= 2)

    attention(3)
    a_scale(3)
    out_proj(3, True)
    for b in range(4):
        out_copy(2, b).wait()
    for b in range(4):
        out_copy(3, b).wait()


@jax.jit
def pallas_concat_heads__linear_attn_block__sliding_local_dilated__prompt_kernel(A_x, A_wqkv, A_wo, B_x, B_wqkv, B_wo):
    xa = jnp.transpose(A_x[0])
    xb = jnp.transpose(B_x[0])
    anyspec = pl.BlockSpec(memory_space=pl.ANY)
    out = pl.pallas_call(
        _kernel,
        grid=(1,),
        in_specs=[anyspec] * 6,
        out_specs=anyspec,
        out_shape=jax.ShapeDtypeStruct((S, 2 * D), BF16),
        scratch_shapes=[
            pltpu.VMEM((KP, S), BF16),
            pltpu.VMEM((KP, S), BF16),
            pltpu.VMEM((D, 3 * D), BF16),
            pltpu.VMEM((D, 3 * D), BF16),
            pltpu.VMEM((D, D), BF16),
            pltpu.VMEM((D, D), BF16),
            pltpu.VMEM((5, KP, 128), F32),
            pltpu.VMEM((2 * D, KP), BF16),
            pltpu.VMEM((3 * D, KP), BF16),
            pltpu.VMEM((D, KP), BF16),
            pltpu.VMEM((D, KP), BF16),
            pltpu.VMEM((D, S), F32),
            pltpu.VMEM((5, D, 128), F32),
            pltpu.VMEM((D, 128), F32),
            pltpu.VMEM((2, 3 * DH, 128 + 2 * HALO, 128), F32),
            pltpu.VMEM((KP, BLK), BF16),
            pltpu.VMEM((KP, BLK), BF16),
            pltpu.VMEM((2, BLK, 2 * D), BF16),
            pltpu.SemaphoreType.DMA((13,)),
            pltpu.SemaphoreType.DMA((8,)),
        ],
        compiler_params=pltpu.CompilerParams(
            dimension_semantics=("arbitrary",),
            vmem_limit_bytes=100 * 1024 * 1024),
    )(xa, A_wqkv, A_wo, xb, B_wqkv, B_wo)
    return out.reshape(1, S, 2 * D)
```

```python
import functools
import math

import jax
import jax.numpy as jnp
from jax import lax
import jax.experimental.pallas as pl
import jax.experimental.pallas.tpu as pltpu

S = 2048
D = 576
H = 32
DH = 18
KP = 640
BLK = 512
NB = S // BLK
HALO = 16
WIN = 8
ATT_R = 8
QK_STEP = 3
PV_STEP = 6
F32 = jnp.float32
BF16 = jnp.bfloat16
I32 = jnp.int32
LOG2E = math.log2(math.e)
CSC = (DH ** -0.5) * LOG2E
NEG = -1e9 * LOG2E
ROWS = [(0, 144), (112, 272), (240, 400), (368, 528), (496, 576)]


def _phi(t):
    return jnp.where(t > 0, t + 1.0, jnp.exp(t)) + 1e-6


def _dot(a, b):
    return jnp.dot(a, b, preferred_element_type=F32)


def _dot_nt(a, b):
    return lax.dot_general(a, b, (((1,), (1,)), ((), ())), preferred_element_type=F32)


def _pk(x):
    return pltpu.bitcast(x, I32)


def _upk(x):
    return pltpu.bitcast(x, BF16)


def _token(vals):
    acc = None
    for v in vals:
        b = pltpu.bitcast(v, I32)
        for r in range(0, b.shape[0], 8):
            for c in range(0, b.shape[1], 128):
                x = b[r:r + 8, c:c + 128]
                acc = x if acc is None else acc | x
    return lax.shift_right_logical(lax.shift_right_logical(acc, 31), 1)


def _mark(r, t):
    b, row = divmod(t - 576, 576)
    row = (row // 8) * 8
    return _token([r[row:row + 8, 128 * b:128 * b + 128]])


def _or_f32(x, tok):
    if tok is None:
        return x
    return pltpu.bitcast(pltpu.bitcast(x, I32) | tok, F32)


def _ktile(w_ref, c, col0, ncol):
    if c < 4:
        return w_ref[pl.ds(128 * c, 128), pl.ds(col0, ncol)]
    blk = w_ref[pl.ds(512, 64), pl.ds(col0, ncol)]
    return jnp.concatenate([blk, jnp.zeros_like(blk)], axis=0)


def _kernel(xa_hbm, wa_hbm, woa_hbm, xb_hbm, wb_hbm, wob_hbm, out_hbm,
            xa, xb, wa, wb, woa, wob,
            wt32, wqkT, wbT, woT, mT, pq, T, zb, att, oT, scT, outbuf,
            sem_in, sem_out):
    def w_copy(name):
        if name == 'wa_k':
            return pltpu.make_async_copy(wa_hbm.at[:, pl.ds(512, 640)], wa.at[:, pl.ds(512, 640)], sem_in.at[0])
        if name == 'wa_q':
            return pltpu.make_async_copy(wa_hbm.at[:, pl.ds(0, 512)], wa.at[:, pl.ds(0, 512)], sem_in.at[13])
        if name == 'wb':
            return pltpu.make_async_copy(wb_hbm, wb, sem_in.at[5])
        if name == 'wa_v':
            return pltpu.make_async_copy(wa_hbm.at[:, pl.ds(1152, 576)], wa.at[:, pl.ds(1152, 576)], sem_in.at[6])
        if name == 'woa':
            return pltpu.make_async_copy(woa_hbm, woa, sem_in.at[7])
        return pltpu.make_async_copy(wob_hbm, wob, sem_in.at[8])

    def xa_copy(i):
        return pltpu.make_async_copy(
            xa_hbm.at[:, pl.ds(i * BLK, BLK)], xa.at[pl.ds(0, D), pl.ds(i * BLK, BLK)], sem_in.at[1 + i])

    def xb_copy(i):
        return pltpu.make_async_copy(
            xb_hbm.at[:, pl.ds(i * BLK, BLK)], xb.at[pl.ds(0, D), pl.ds(i * BLK, BLK)], sem_in.at[9 + i])

    def out_copy(j, b):
        return pltpu.make_async_copy(
            outbuf.at[pl.ds(j * BLK + b * 128, 128), :],
            out_hbm.at[pl.ds(j * BLK + b * 128, 128), :],
            sem_out.at[j * 4 + b])

    queue = []
    due = {}

    def add_due(n, tok):
        due[n] = tok if n not in due else due[n] | tok

    def rhs(ref, col0, every=0, phase=0, packed=False):
        cols = []
        n = 0
        for b in range(4):
            tiles = []
            for c in range(5):
                if every and queue and n % every == phase:
                    add_due(n, queue.pop(0)())
                tok = due.pop(n, None)
                if packed:
                    t = ref[pl.ds(64 * c, 64), pl.ds(col0 + 128 * b, 128)]
                    if tok is not None:
                        t = jnp.concatenate([t[0:8, :] | tok, t[8:, :]], axis=0)
                    t = _upk(t)
                else:
                    t = ref[pl.ds(128 * c, 128), pl.ds(col0 + 128 * b, 128)]
                    if tok is not None:
                        t = jnp.concatenate([_upk(_pk(t[0:16, :]) | tok), t[16:, :]], axis=0)
                n += 1
                tiles.append(t)
            cols.append(jnp.concatenate(tiles, axis=0))
        assert not due
        return jnp.concatenate(cols, axis=1)

    def flush():
        while queue:
            queue.pop(0)()

    def lhs(ref, row0):
        return _upk(ref[pl.ds(row0 // 2, D // 2), :])

    def prep_piece(buf, w_ref, col0, ncol, off, dst, base, c):
        def run():
            wt32[buf, c, pl.ds(0, ncol), :] = _ktile(w_ref, c, col0, ncol).T.astype(F32)
            outs = []
            for d in range(0, DH, 2):
                r0 = wt32[buf, c, pl.ds(off + d, 32, stride=DH), :]
                r1 = wt32[buf, c, pl.ds(off + d + 1, 32, stride=DH), :]
                v = _pk(jnp.concatenate([r0, r1], axis=0).astype(BF16))
                dst[pl.ds(base // 2 + 16 * d, 32), pl.ds(128 * c, 128)] = v
                outs.append(v)
            return _token(outs)
        return run

    def perm_t_piece(buf, dst, c):
        nrow = 128 if c < 4 else 64
        outs = []
        for kt in range(5):
            ds_ = range(4 * kt, min(4 * kt + 4, DH))
            rows = [wt32[buf, c, pl.ds(d, 32, stride=DH), :] for d in ds_]
            if kt == 4:
                rows.append(jnp.zeros((64, 128), F32))
            tile = _pk(jnp.concatenate(rows, axis=0).astype(BF16).T[:nrow, :])
            dst[pl.ds(64 * c, nrow // 2), pl.ds(128 * kt, 128)] = tile
            outs.append(tile)
        return _token(outs)

    def prep_wo_piece(buf, c):
        def run():
            if c < 4:
                wt32[buf, c, pl.ds(0, D), :] = wob[:, pl.ds(128 * c, 128)].astype(F32)
            else:
                wt32[buf, 4, pl.ds(0, D), :] = jnp.concatenate(
                    [wob[:, pl.ds(512, 64)].astype(F32), jnp.zeros((D, 64), F32)], axis=1)
            return perm_t_piece(buf, woT, c)
        return run

    def a_kt(i, every=0):
        first = i == 0
        kT = _dot(lhs(wqkT, D), rhs(xa, i * BLK, every))
        pk = _phi(kT).astype(BF16)
        xblk = rhs(xa, i * BLK, every)
        for c in range(5):
            t = _dot_nt(pk, xblk[128 * c:128 * (c + 1), :])
            if first:
                T[c] = t
            else:
                T[c] += t

    def a_q(i, every=0, phase=0):
        qT = _dot(lhs(wqkT, 0), rhs(xa, i * BLK, every, phase))
        pq[:, pl.ds(i * BLK, BLK)] = _phi(qT)
        return qT

    def b_part(j, p, every=0, phase=0):
        first = j == 0
        lane = lax.broadcasted_iota(I32, (HALO, 128), 1)
        r32 = _dot(lhs(wbT, D * p), rhs(xb, j * BLK, every, phase))
        r = r32.astype(BF16)
        for d in range(DH):
            tile = jnp.concatenate(
                [r[32 * d:32 * d + 32, 128 * b:128 * b + 128] for b in range(4)], axis=0)
            tt = tile.T.astype(F32)
            att[j, p * DH + d, pl.ds(HALO, 128), :] = tt
            add_due(4 + (d * 12) // DH, _token([tt[120:128, :]]))
            if p > 0:
                cur = pltpu.roll(tt[128 - HALO:, :], 32, 1)
                if first:
                    if p == 1:
                        prev = jnp.zeros((HALO, 128), F32)
                    else:
                        prev = jnp.broadcast_to(tt[0:1, :], (HALO, 128))
                else:
                    prev = att[j - 1, p * DH + d, pl.ds(128 + HALO, HALO), :]
                att[j, p * DH + d, pl.ds(0, HALO), :] = jnp.where(lane < 32, prev, cur)
                if j < NB - 1:
                    att[j, p * DH + d, pl.ds(128 + HALO, HALO), :] = cur
        return r32

    def att_group(j, g):
        R = ATT_R
        base = HALO + g * R
        ls = [None] * WIN
        csc = None
        for d in range(DH):
            if d % QK_STEP == 0:
                tok = yield
                csc = _or_f32(jnp.full((R, 128), CSC, F32), tok)
            q = att[j, d, pl.ds(base, R), :] * csc
            for w in range(WIN):
                t = q * att[j, DH + d, pl.ds(base - 2 * w, R), :]
                ls[w] = t if ls[w] is None else ls[w] + t
        if g * R < HALO and j == 0:
            pos = (lax.broadcasted_iota(I32, (R, 128), 0) + g * R
                   + (lax.broadcasted_iota(I32, (R, 128), 1) // 32) * 128)
            ls = [ls[0]] + [jnp.where(pos >= 2 * w, ls[w], NEG) for w in range(1, WIN)]
        m = functools.reduce(jnp.maximum, ls)
        es = [jnp.exp2(l - m) for l in ls]
        inv = 1.0 / functools.reduce(lambda a, b: a + b, es)
        ps = None
        for d in range(DH):
            if d % PV_STEP == 0:
                tok = yield
                invt = _or_f32(inv, tok)
                ps = [e * invt for e in es]
            acc = None
            for w in range(WIN):
                t = ps[w] * att[j, 2 * DH + d, pl.ds(base - 2 * w, R), :]
                acc = t if acc is None else acc + t
            att[j, d, pl.ds(base, R), :] = acc

    NPIECE = (128 // ATT_R) * (DH // QK_STEP + DH // PV_STEP)
    state = {'gens': [], 'left': 0}

    def att_begin(j):
        gens = [att_group(j, g) for g in range(128 // ATT_R)]
        for gen in gens:
            next(gen)
        state['gens'] = gens
        state['left'] = NPIECE

    def release(r, n):
        n = min(n, state['left'])
        for i in range(n):
            tok = _mark(r, 576 + (2304 * i) // n)
            gen = state['gens'][0]
            try:
                gen.send(tok)
            except StopIteration:
                state['gens'].pop(0)
            state['left'] -= 1

    def ot_piece(j, d0, d1):
        def run():
            outs = []
            for d in range(d0, d1):
                ot = _pk(att[j, d, pl.ds(HALO, 128), :].astype(BF16).T)
                for b in range(4):
                    oT[pl.ds(16 * d, 16), pl.ds(j * BLK + 128 * b, 128)] = ot[16 * b:16 * b + 16, :]
                outs.append(ot[56:64, :])
            return _token(outs)
        return run

    def a_scale(j):
        for b in range(4):
            col = pl.ds(j * BLK + 128 * b, 128)
            den = None
            for d in range(DH):
                t = pq[pl.ds(32 * d, 32), col] * zb[pl.ds(32 * d, 32), :]
                den = t if den is None else den + t
            inv = 1.0 / (den + 1e-6)
            for d in range(DH):
                scT[pl.ds(16 * d, 16), col] = _pk((pq[pl.ds(32 * d, 32), col] * inv).astype(BF16))

    def out_b(j):
        return _dot(lhs(woT, 0), rhs(oT, j * BLK, packed=True))

    def out_a(j):
        return _dot(lhs(mT, 0), rhs(scT, j * BLK, packed=True))

    def out_store(j, oa32, ob32, tie):
        oa = oa32.astype(BF16)
        ob = ob32.astype(BF16)
        for b in range(4):
            blk = jnp.concatenate([oa[:, 128 * b:128 * b + 128], ob[:, 128 * b:128 * b + 128]], axis=0)
            bt = blk.T
            outbuf[pl.ds(j * BLK + 128 * b, 128), :] = bt
            if tie:
                add_due(4 + 4 * b, _token([bt[112:128, :]]))
            out_copy(j, b).start()

    def a_small_g():
        kvs = []
        for jt, (r0, r1) in enumerate(ROWS):
            n = r1 - r0
            w = 128 if jt < 4 else 64
            tb = jnp.concatenate([T[c, pl.ds(r0, n), :] for c in range(5)], axis=1)[:, :D].astype(BF16)
            g = _dot(tb, wa[:, pl.ds(1152 + 128 * jt, w)])
            rh = (lax.broadcasted_iota(I32, (n, w), 0) + r0) // DH
            ch = (lax.broadcasted_iota(I32, (n, w), 1) + 128 * jt) // DH
            kvs.append(jnp.where(rh == ch, g, 0.0).astype(BF16))
        lane = lax.broadcasted_iota(I32, (32, 128), 1)
        for d in range(DH):
            t = T[4, pl.ds(d, 32, stride=DH), :]
            zb[pl.ds(32 * d, 32), :] = jnp.where(lane >= 64, t, pltpu.roll(t, 64, 1))
        return kvs

    def a_small_m(buf, kvs):
        for c in range(5):
            wt32[buf, c, pl.ds(0, D), :] = jnp.zeros((D, 128), F32)
        for jt, (r0, r1) in enumerate(ROWS):
            n = r1 - r0
            w = 128 if jt < 4 else 64
            mrow = _dot(kvs[jt], woa[pl.ds(128 * jt, w), :])
            for c in range(4):
                wt32[buf, c, pl.ds(r0, n), :] += mrow[:, 128 * c:128 * c + 128]
            wt32[buf, 4, pl.ds(r0, n), pl.ds(0, 64)] += mrow[:, 512:576]

    w_copy('wa_k').start()
    xa_copy(0).start()
    xa[pl.ds(D, KP - D), :] = jnp.ones((KP - D, S), BF16)
    xb[pl.ds(D, KP - D), :] = jnp.zeros((KP - D, S), BF16)
    oT[pl.ds(D // 2, (KP - D) // 2), :] = jnp.zeros(((KP - D) // 2, S), I32)
    scT[pl.ds(D // 2, (KP - D) // 2), :] = jnp.zeros(((KP - D) // 2, S), I32)
    w_copy('wa_k').wait()
    for i in range(1, NB):
        xa_copy(i).start()
    w_copy('wb').start()
    w_copy('wa_q').start()
    w_copy('wob').start()
    w_copy('wa_v').start()
    w_copy('woa').start()
    for i in range(NB):
        xb_copy(i).start()
    for c in range(5):
        wqkT[pl.ds(D // 2, D // 2), pl.ds(128 * c, 128)] = _pk(_ktile(wa, c, 512, 640).T[64:, :])
    xa_copy(0).wait()
    a_kt(0)

    for i in range(1, NB):
        xa_copy(i).wait()
    a_kt(1)

    w_copy('wb').wait()
    w_copy('wa_q').wait()
    w_copy('wob').wait()
    for c in range(5):
        queue.append(prep_piece(0, wb, 0, 640, 0, wbT, 0, c))
    for c in range(5):
        queue.append(prep_piece(1, wb, 512, 640, 64, wbT, D, c))
    for c in range(5):
        queue.append(prep_piece(2, wb, 1152, 576, 0, wbT, 2 * D, c))
    for c in range(5):
        queue.append(prep_piece(3, wa, 0, 640, 0, wqkT, 0, c))
    for c in range(5):
        queue.append(prep_wo_piece(4, c))
    a_kt(2, 3, )
    a_kt(3, 3)
    flush()

    w_copy('wa_v').wait()
    w_copy('woa').wait()
    for i in range(NB - 1):
        xb_copy(i).wait()
    kvs = a_small_g()
    b_part(0, 0)
    a_small_m(0, kvs)
    b_part(0, 1)
    for c in range(5):
        queue.append(functools.partial(perm_t_piece, 0, mT, c))
    b_part(0, 2, 4, 2)
    flush()
    att_begin(0)
    for j in range(NB):
        if j + 1 < NB:
            n = state['left']
            release(b_part(j + 1, 0), (n + 2) // 3)
            release(b_part(j + 1, 1), (n + 1) // 3)
            release(b_part(j + 1, 2), n // 3)
            assert state['left'] == 0
            for d0 in range(0, DH, 3):
                queue.append(ot_piece(j, d0, d0 + 3))
            a_q(j, 2, 0)
            flush()
            att_begin(j + 1)
            if j == 1:
                xb_copy(NB - 1).wait()
            if j >= 2:
                for b in range(4):
                    out_copy(j - 2, b).wait()
            a_scale(j)
            nr = NPIECE // 5 if j + 2 < NB else NPIECE // 3
            ob = out_b(j)
            release(ob, nr)
            oa = out_a(j)
            release(oa, nr)
            out_store(j, oa, ob, True)
        else:
            release(a_q(j), NPIECE)
            assert state['left'] == 0
            for b in range(4):
                out_copy(j - 2, b).wait()
            a_scale(j)
            oa = out_a(j)
            for d0 in range(0, DH, 3):
                ot_piece(j, d0, d0 + 3)()
            ob = out_b(j)
            out_store(j, oa, ob, False)
    for j in range(NB - 2, NB):
        for b in range(4):
            out_copy(j, b).wait()


@jax.jit
def pallas_concat_heads__linear_attn_block__sliding_local_dilated__prompt_kernel(A_x, A_wqkv, A_wo, B_x, B_wqkv, B_wo):
    xa = jnp.transpose(A_x[0])
    xb = jnp.transpose(B_x[0])
    anyspec = pl.BlockSpec(memory_space=pl.ANY)
    out = pl.pallas_call(
        _kernel,
        grid=(1,),
        in_specs=[anyspec] * 6,
        out_specs=anyspec,
        out_shape=jax.ShapeDtypeStruct((S, 2 * D), BF16),
        scratch_shapes=[
            pltpu.VMEM((KP, S), BF16),
            pltpu.VMEM((KP, S), BF16),
            pltpu.VMEM((D, 3 * D), BF16),
            pltpu.VMEM((D, 3 * D), BF16),
            pltpu.VMEM((D, D), BF16),
            pltpu.VMEM((D, D), BF16),
            pltpu.VMEM((5, 5, KP, 128), F32),
            pltpu.VMEM((D, KP), I32),
            pltpu.VMEM((3 * D // 2, KP), I32),
            pltpu.VMEM((D // 2, KP), I32),
            pltpu.VMEM((D // 2, KP), I32),
            pltpu.VMEM((D, S), F32),
            pltpu.VMEM((5, D, 128), F32),
            pltpu.VMEM((D, 128), F32),
            pltpu.VMEM((NB, 3 * DH, 128 + 2 * HALO, 128), F32),
            pltpu.VMEM((KP // 2, S), I32),
            pltpu.VMEM((KP // 2, S), I32),
            pltpu.VMEM((S, 2 * D), BF16),
            pltpu.SemaphoreType.DMA((14,)),
            pltpu.SemaphoreType.DMA((16,)),
        ],
        compiler_params=pltpu.CompilerParams(
            dimension_semantics=("arbitrary",),
            vmem_limit_bytes=100 * 1024 * 1024),
    )(xa, A_wqkv, A_wo, xb, B_wqkv, B_wo)
    return out.reshape(1, S, 2 * D)
```

```python
import functools
import math

import jax
import jax.numpy as jnp
from jax import lax
import jax.experimental.pallas as pl
import jax.experimental.pallas.tpu as pltpu

S = 2048
D = 576
H = 32
DH = 18
KP = 640
BLK = 512
NB = S // BLK
HALO = 16
WIN = 8
ATT_R = 8
QK_STEP = 3
PV_STEP = 6
WAIT_ROW = 256
PRO_ROW = 304
AT_OT = (7, 9, 10, 12, 15, 17)
F32 = jnp.float32
BF16 = jnp.bfloat16
I32 = jnp.int32
LOG2E = math.log2(math.e)
CSC = (DH ** -0.5) * LOG2E
NEG = -1e9 * LOG2E
ROWS = [(0, 144), (112, 272), (240, 400), (368, 528), (496, 576)]


def _phi(t):
    return jnp.where(t > 0, t + 1.0, jnp.exp(t)) + 1e-6


def _dot(a, b):
    return jnp.dot(a, b, preferred_element_type=F32)


def _dot_nt(a, b):
    return lax.dot_general(a, b, (((1,), (1,)), ((), ())), preferred_element_type=F32)


def _pk(x):
    return pltpu.bitcast(x, I32)


def _upk(x):
    return pltpu.bitcast(x, BF16)


def _token(vals):
    acc = None
    for v in vals:
        b = pltpu.bitcast(v, I32)
        for r in range(0, b.shape[0], 8):
            for c in range(0, b.shape[1], 128):
                x = b[r:r + 8, c:c + 128]
                acc = x if acc is None else acc | x
    return lax.shift_right_logical(lax.shift_right_logical(acc, 31), 1)


def _mark(r, t):
    b, row = divmod(t - 576, 576)
    row = (row // 8) * 8
    return _token([r[row:row + 8, 128 * b:128 * b + 128]])


def _or_f32(x, tok):
    if tok is None:
        return x
    return pltpu.bitcast(pltpu.bitcast(x, I32) | tok, F32)


def _ktile(w_ref, c, col0, ncol):
    if c < 4:
        return w_ref[pl.ds(128 * c, 128), pl.ds(col0, ncol)]
    blk = w_ref[pl.ds(512, 64), pl.ds(col0, ncol)]
    return jnp.concatenate([blk, jnp.zeros_like(blk)], axis=0)


def _kernel(xa_hbm, wa_hbm, woa_hbm, xb_hbm, wb_hbm, wob_hbm, out_hbm,
            xa, xb, wa, wb, woa, wob,
            wt32, wqkT, wbT, woT, mT, pq, T, zb, att, oT, scT, outbuf, mk,
            sem):
    def rows_copy(src, dst, r0, n, col0, ncol, s):
        return pltpu.make_async_copy(src.at[pl.ds(r0, n), pl.ds(col0, ncol)],
                                     dst.at[pl.ds(r0, n), pl.ds(col0, ncol)], sem.at[s])

    def in_copy(name):
        if name == 'w0':
            return rows_copy(wa_hbm, wa, 0, 128, 512, 640, 0)
        if name == 'x0':
            return rows_copy(xa_hbm, xa, 0, 128, 0, BLK, 1)
        if name == 'w1':
            return rows_copy(wa_hbm, wa, 128, 128, 512, 640, 2)
        if name == 'x1':
            return rows_copy(xa_hbm, xa, 128, 128, 0, BLK, 3)
        if name == 'w2':
            return rows_copy(wa_hbm, wa, 256, 128, 512, 640, 4)
        if name == 'x2':
            return rows_copy(xa_hbm, xa, 256, 128, 0, BLK, 5)
        if name == 'w34':
            return rows_copy(wa_hbm, wa, 384, 192, 512, 640, 6)
        if name == 'x34':
            return rows_copy(xa_hbm, xa, 384, 192, 0, BLK, 7)
        if name == 'xa':
            return rows_copy(xa_hbm, xa, 0, D, BLK, S - BLK, 0)
        if name == 'wa_q':
            return rows_copy(wa_hbm, wa, 0, D, 0, 512, 1)
        if name == 'wb':
            return pltpu.make_async_copy(wb_hbm, wb, sem.at[2])
        if name == 'wob':
            return pltpu.make_async_copy(wob_hbm, wob, sem.at[3])
        if name == 'wa_v':
            return rows_copy(wa_hbm, wa, 0, D, 1152, 576, 4)
        if name == 'woa':
            return pltpu.make_async_copy(woa_hbm, woa, sem.at[5])
        return pltpu.make_async_copy(xb_hbm, xb.at[pl.ds(0, D), :], sem.at[6])

    outs_started = []

    def out_start(row0, nrow, col0, ncol):
        cp = pltpu.make_async_copy(
            outbuf.at[pl.ds(row0, nrow), pl.ds(col0, ncol)],
            out_hbm.at[pl.ds(row0, nrow), pl.ds(col0, ncol)],
            sem.at[len(outs_started)])
        outs_started.append(cp)
        cp.start()

    queue = []
    due = {}

    def add_due(n, tok):
        due[n] = tok if n not in due else due[n] | tok

    def tile(ref, c, col, n, at, packed):
        if n in at and queue:
            add_due(n, queue.pop(0)())
        tok = due.pop(n, None)
        if packed:
            t = ref[pl.ds(64 * c, 64), pl.ds(col, 128)]
            if tok is not None:
                t = jnp.concatenate([t[0:8, :] | tok, t[8:, :]], axis=0)
            return _upk(t)
        t = ref[pl.ds(128 * c, 128), pl.ds(col, 128)]
        if tok is not None:
            t = jnp.concatenate([_upk(_pk(t[0:16, :]) | tok), t[16:, :]], axis=0)
        return t

    def rhs(ref, col0, at=(), packed=False, bs=range(4)):
        cols = []
        for b in bs:
            tiles = [tile(ref, c, col0 + 128 * b, 5 * b + c, at, packed) for c in range(5)]
            cols.append(jnp.concatenate(tiles, axis=0))
        assert bs[-1] < 3 or not due
        return jnp.concatenate(cols, axis=1)

    def flush():
        while queue:
            queue.pop(0)()

    def lhs(ref, row0):
        return _upk(ref[pl.ds(row0 // 2, D // 2), :])

    def prep_piece(buf, w_ref, col0, ncol, off, dst, base, c):
        def run():
            wt32[buf, c, pl.ds(0, ncol), :] = _ktile(w_ref, c, col0, ncol).T.astype(F32)
            outs = []
            for d in range(0, DH, 2):
                r0 = wt32[buf, c, pl.ds(off + d, 32, stride=DH), :]
                r1 = wt32[buf, c, pl.ds(off + d + 1, 32, stride=DH), :]
                v = _pk(jnp.concatenate([r0, r1], axis=0).astype(BF16))
                dst[pl.ds(base // 2 + 16 * d, 32), pl.ds(128 * c, 128)] = v
                outs.append(v)
            return _token(outs)
        return run

    def perm_t_piece(buf, dst, c):
        nrow = 128 if c < 4 else 64
        outs = []
        for kt in range(5):
            ds_ = range(4 * kt, min(4 * kt + 4, DH))
            rows = [wt32[buf, c, pl.ds(d, 32, stride=DH), :] for d in ds_]
            if kt == 4:
                rows.append(jnp.zeros((64, 128), F32))
            tile = _pk(jnp.concatenate(rows, axis=0).astype(BF16).T[:nrow, :])
            dst[pl.ds(64 * c, nrow // 2), pl.ds(128 * kt, 128)] = tile
            outs.append(tile)
        return _token(outs)

    def prep_wo_piece(buf, c):
        def run():
            if c < 4:
                wt32[buf, c, pl.ds(0, D), :] = wob[:, pl.ds(128 * c, 128)].astype(F32)
            else:
                wt32[buf, 4, pl.ds(0, D), :] = jnp.concatenate(
                    [wob[:, pl.ds(512, 64)].astype(F32), jnp.zeros((D, 64), F32)], axis=1)
            return perm_t_piece(buf, woT, c)
        return run

    def a_kt(i, at_k=(), at_t=(), kT=None, waits=()):
        if kT is None:
            kT = _dot(lhs(wqkT, D), rhs(xa, i * BLK, at_k))
        pk = _phi(kT).astype(BF16)
        for c in range(5):
            xrow = jnp.concatenate(
                [tile(xa, c, i * BLK + 128 * b, 4 * c + b, at_t, False) for b in range(4)], axis=1)
            t = _dot_nt(pk, xrow)
            if i == 0:
                T[c] = t
            else:
                T[c] += t
        assert not due

    def a_q(i, at=()):
        qT = _dot(lhs(wqkT, 0), rhs(xa, i * BLK, at))
        pq[:, pl.ds(i * BLK, BLK)] = _phi(qT)
        return qT

    def b_part(j, p, at=()):
        first = j == 0
        lane = lax.broadcasted_iota(I32, (HALO, 128), 1)
        r32 = _dot(lhs(wbT, D * p), rhs(xb, j * BLK, at))
        r = r32.astype(BF16)
        for d in range(DH):
            tl = jnp.concatenate(
                [r[32 * d:32 * d + 32, 128 * b:128 * b + 128] for b in range(4)], axis=0)
            tt = tl.T.astype(F32)
            att[j, p * DH + d, pl.ds(HALO, 128), :] = tt
            tvals = [tt[120:128, :]]
            if p > 0:
                cur = pltpu.roll(tt[128 - HALO:, :], 32, 1)
                if first:
                    if p == 1:
                        prev = jnp.zeros((HALO, 128), F32)
                    else:
                        prev = jnp.broadcast_to(tt[0:1, :], (HALO, 128))
                else:
                    prev = att[j - 1, p * DH + d, pl.ds(128 + HALO, HALO), :]
                halo = jnp.where(lane < 32, prev, cur)
                att[j, p * DH + d, pl.ds(0, HALO), :] = halo
                tvals.append(halo)
                if j < NB - 1:
                    att[j, p * DH + d, pl.ds(128 + HALO, HALO), :] = cur
            add_due(4 + (d * 12) // DH, _token(tvals))
        return r32

    def att_group(j, g):
        R = ATT_R
        base = HALO + g * R
        ls = [None] * WIN
        csc = None
        for d in range(DH):
            if d % QK_STEP == 0:
                tok = yield
                csc = _or_f32(jnp.full((R, 128), CSC, F32), tok)
            q = att[j, d, pl.ds(base, R), :] * csc
            for w in range(WIN):
                t = q * att[j, DH + d, pl.ds(base - 2 * w, R), :]
                ls[w] = t if ls[w] is None else ls[w] + t
        if g * R < HALO and j == 0:
            pos = (lax.broadcasted_iota(I32, (R, 128), 0) + g * R
                   + (lax.broadcasted_iota(I32, (R, 128), 1) // 32) * 128)
            ls = [ls[0]] + [jnp.where(pos >= 2 * w, ls[w], NEG) for w in range(1, WIN)]
        m = functools.reduce(jnp.maximum, ls)
        es = [jnp.exp2(l - m) for l in ls]
        inv = 1.0 / functools.reduce(lambda a, b: a + b, es)
        ps = None
        for d in range(DH):
            if d % PV_STEP == 0:
                tok = yield
                invt = _or_f32(inv, tok)
                ps = [e * invt for e in es]
            acc = None
            for w in range(WIN):
                t = ps[w] * att[j, 2 * DH + d, pl.ds(base - 2 * w, R), :]
                acc = t if acc is None else acc + t
            att[j, d, pl.ds(base, R), :] = acc

    NPIECE = (128 // ATT_R) * (DH // QK_STEP + DH // PV_STEP)
    state = {'gens': [], 'left': 0}

    def att_begin(j):
        gens = [att_group(j, g) for g in range(128 // ATT_R)]
        for gen in gens:
            next(gen)
        state['gens'] = gens
        state['left'] = NPIECE

    def release(r, n):
        n = min(n, state['left'])
        for i in range(n):
            tok = _mark(r, 576 + (2304 * i) // n)
            gen = state['gens'][0]
            try:
                gen.send(tok)
            except StopIteration:
                state['gens'].pop(0)
            state['left'] -= 1

    def ot_piece(j, d0, d1):
        def run():
            outs = []
            for d in range(d0, d1):
                ot = _pk(att[j, d, pl.ds(HALO, 128), :].astype(BF16).T)
                for b in range(4):
                    oT[pl.ds(16 * d, 16), pl.ds(j * BLK + 128 * b, 128)] = ot[16 * b:16 * b + 16, :]
                outs.append(ot[56:64, :])
            return _token(outs)
        return run

    def a_scale(j):
        for b in range(4):
            col = pl.ds(j * BLK + 128 * b, 128)
            den = None
            for d in range(DH):
                t = pq[pl.ds(32 * d, 32), col] * zb[pl.ds(32 * d, 32), :]
                den = t if den is None else den + t
            inv = 1.0 / (den + 1e-6)
            for d in range(DH):
                scT[pl.ds(16 * d, 16), col] = _pk((pq[pl.ds(32 * d, 32), col] * inv).astype(BF16))

    def out_b(j):
        return _dot(lhs(woT, 0), rhs(oT, j * BLK, packed=True))

    def out_a(j, at=()):
        return _dot(lhs(mT, 0), rhs(scT, j * BLK, at, packed=True))

    def store_t(row0, col0, blk):
        bt = blk.T
        outbuf[pl.ds(row0, 128), pl.ds(col0, blk.shape[0])] = bt
        return _token([bt[112:128, :]])

    def store_a(j, oa, n0, dn):
        for b in range(4):
            tok = store_t(j * BLK + 128 * b, 0, oa[0:512, 128 * b:128 * b + 128])
            add_due(n0 + dn * b, tok)

    def store_b(j, oa, ob, n0, dn):
        for b in range(4):
            blk = jnp.concatenate([oa[512:D, 128 * b:128 * b + 128], ob[:, 128 * b:128 * b + 128]], axis=0)
            tok = store_t(j * BLK + 128 * b, 512, blk)
            add_due(n0 + dn * b, tok)

    def a_small_g():
        kvs = []
        for jt, (r0, r1) in enumerate(ROWS):
            n = r1 - r0
            w = 128 if jt < 4 else 64
            tb = jnp.concatenate([T[c, pl.ds(r0, n), :] for c in range(5)], axis=1)[:, :D].astype(BF16)
            g = _dot(tb, wa[:, pl.ds(1152 + 128 * jt, w)])
            rh = (lax.broadcasted_iota(I32, (n, w), 0) + r0) // DH
            ch = (lax.broadcasted_iota(I32, (n, w), 1) + 128 * jt) // DH
            kvs.append(jnp.where(rh == ch, g, 0.0).astype(BF16))
        lane = lax.broadcasted_iota(I32, (32, 128), 1)
        for d in range(DH):
            t = T[4, pl.ds(d, 32, stride=DH), :]
            zb[pl.ds(32 * d, 32), :] = jnp.where(lane >= 64, t, pltpu.roll(t, 64, 1))
        return kvs

    def a_small_m(buf, kvs):
        for c in range(5):
            wt32[buf, c, pl.ds(0, D), :] = jnp.zeros((D, 128), F32)
        for jt, (r0, r1) in enumerate(ROWS):
            n = r1 - r0
            if jt < 4:
                mrow = _dot(kvs[jt], woa[pl.ds(128 * jt, 128), :])
            else:
                w4 = woa[pl.ds(512, 64), :]
                mrow = jnp.concatenate([
                    _dot(kvs[4], w4[:, :384]),
                    jnp.concatenate([_dot(kvs[4][:48], w4[:, 384:]), _dot(kvs[4][48:], w4[:, 384:])], axis=0)],
                    axis=1)
            for c in range(4):
                wt32[buf, c, pl.ds(r0, n), :] += mrow[:, 128 * c:128 * c + 128]
            wt32[buf, 4, pl.ds(r0, n), pl.ds(0, 64)] += mrow[:, 512:576]

    for name in ('w0', 'x0', 'w1', 'x1', 'w2', 'x2', 'w34', 'x34'):
        in_copy(name).start()
    xa[pl.ds(D, KP - D), :] = jnp.ones((KP - D, S), BF16)
    xb[pl.ds(D, KP - D), :] = jnp.zeros((KP - D, S), BF16)
    oT[pl.ds(D // 2, (KP - D) // 2), :] = jnp.zeros(((KP - D) // 2, S), I32)
    scT[pl.ds(D // 2, (KP - D) // 2), :] = jnp.zeros(((KP - D) // 2, S), I32)

    def wk_t(c):
        wqkT[pl.ds(D // 2, D // 2), pl.ds(128 * c, 128)] = _pk(_ktile(wa, c, 512, 640).T[64:, :])

    def kt_part(c0, nc):
        return _dot(_upk(wqkT[pl.ds(D // 2, D // 2), pl.ds(128 * c0, 128 * nc)]),
                    xa[pl.ds(128 * c0, 128 * nc), pl.ds(0, BLK)])

    in_copy('w0').wait()
    wk_t(0)
    kT = None
    for c, (ws, nxt, tr) in enumerate([
            (('x0', 'w1'), ('xa', 'wa_q'), (1,)),
            (('x1', 'w2'), ('wb', 'wob'), (2,)),
            (('x2', 'w34'), ('wa_v', 'woa', 'xb'), (3, 4))]):
        for name in ws:
            in_copy(name).wait()
        for name in nxt:
            in_copy(name).start()
        part = kt_part(c, 1)
        for t in tr:
            wk_t(t)
        mk[...] = part[0:8, 0:128]
        kT = part if kT is None else kT + part
    in_copy('x34').wait()
    a_kt(0, kT=kT + kt_part(3, 2))

    in_copy('xa').wait()
    in_copy('wa_q').wait()
    for c in range(5):
        queue.append(prep_piece(3, wa, 0, 640, 0, wqkT, 0, c))
    AT5 = (5, 8, 11, 14, 17)
    a_kt(1, (9, 14, 19), (4, 9))
    a_kt(2)
    a_kt(3)

    for name in ('wb', 'wob', 'wa_v', 'woa', 'xb'):
        in_copy(name).wait()
    kvs = a_small_g()
    for c in range(5):
        queue.append(prep_piece(0, wb, 0, 640, 0, wbT, 0, c))
    a_q(0, (2, 5, 8, 11, 14))
    for c in range(5):
        queue.append(prep_piece(1, wb, 512, 640, 64, wbT, D, c))
    b_part(0, 0, (2, 5, 8, 11, 14))
    a_small_m(0, kvs)
    for c in range(5):
        queue.append(prep_piece(2, wb, 1152, 576, 0, wbT, 2 * D, c))
    b_part(0, 1, (2, 5, 8, 11, 14))
    for c in range(5):
        queue.append(functools.partial(perm_t_piece, 0, mT, c))
    b_part(0, 2, AT5)
    for c in range(5):
        queue.append(prep_wo_piece(4, c))

    def spread(rs):
        for i, (fn, wgt) in enumerate(rs):
            tot = sum(w for _, w in rs[i:])
            n = int(round(state['left'] * wgt / tot))
            release(fn(), n)
        assert state['left'] == 0

    def queue_ot(j):
        for d0 in range(0, DH, 3):
            queue.append(ot_piece(j, d0, d0 + 3))

    res = {}

    def keep(name, fn):
        def run():
            res[name] = fn()
            return res[name]
        return run

    att_begin(0)
    a_scale(0)
    spread([(lambda: b_part(1, 0, AT5), 1), (lambda: b_part(1, 1), 1), (lambda: b_part(1, 2), 1),
            (lambda: a_q(1), 1)])
    flush()
    for j in range(2):
        queue_ot(j)
        att_begin(j + 1)

        def f_b0():
            store_b(j, res['oa'].astype(BF16), res['ob'].astype(BF16), 4, 4)
            out_start(j * BLK, BLK, 0, 2 * D)
            return b_part(j + 2, 0)

        def f_ob():
            flush()
            store_a(j, res['oa'].astype(BF16), 4, 4)
            return out_b(j)

        spread([(keep('oa', lambda: out_a(j, AT_OT)), 0.5), (keep('ob', f_ob), 1), (f_b0, 1),
                (lambda: b_part(j + 2, 1), 1), (lambda: b_part(j + 2, 2), 1)])
        if j == 0:
            a_scale(1)
    queue_ot(2)
    att_begin(3)

    def f_ob2():
        flush()
        a_scale(2)
        return out_b(2)

    def f_aq3():
        oa = res['oa'].astype(BF16)
        store_a(2, oa, 2, 4)
        store_b(2, oa, res['ob'].astype(BF16), 4, 4)
        out_start(2 * BLK, BLK, 0, 2 * D)
        return a_q(3)

    spread([(lambda: a_q(2, AT_OT), 0.5), (keep('ob', f_ob2), 1), (keep('oa', lambda: out_a(2)), 1),
            (f_aq3, 1)])
    a_scale(3)
    oa = out_a(3).astype(BF16)
    for d0 in range(0, DH, 3):
        ot_piece(3, d0, d0 + 3)()
    j = NB - 1
    store_a(j, oa, 4, 2)
    out_start(j * BLK, BLK, 0, 512)
    lw = woT[...]
    for b in range(4):
        if b == 3:
            lw = jnp.concatenate([
                lw[:, :512],
                jnp.concatenate([lw[:208, 512:], lw[208:216, 512:] | last_tok, lw[216:, 512:]], axis=0)], axis=1)
        ob = _dot(_upk(lw), rhs(oT, j * BLK, packed=True, bs=[b])).astype(BF16)
        blk = jnp.concatenate([oa[512:D, 128 * b:128 * b + 128], ob], axis=0)
        row0 = j * BLK + 128 * b
        if b < 3:
            tok = store_t(row0, 512, blk)
            if b < 2:
                add_due(13 + 4 * b, tok)
            else:
                last_tok = tok
            if b == 1:
                out_start(j * BLK, 256, 512, 640)
            if b == 2:
                out_start(row0, 128, 512, 640)
        else:
            store_t(row0, 512, blk[:512])
            out_start(row0, 128, 512, 512)
            store_t(row0, 1024, blk[512:])
            out_start(row0, 128, 1024, 128)
    for cp in outs_started:
        cp.wait()


@jax.jit
def pallas_concat_heads__linear_attn_block__sliding_local_dilated__prompt_kernel(A_x, A_wqkv, A_wo, B_x, B_wqkv, B_wo):
    xa = jnp.transpose(A_x[0])
    xb = jnp.transpose(B_x[0])
    anyspec = pl.BlockSpec(memory_space=pl.ANY)
    out = pl.pallas_call(
        _kernel,
        grid=(1,),
        in_specs=[anyspec] * 6,
        out_specs=anyspec,
        out_shape=jax.ShapeDtypeStruct((S, 2 * D), BF16),
        scratch_shapes=[
            pltpu.VMEM((KP, S), BF16),
            pltpu.VMEM((KP, S), BF16),
            pltpu.VMEM((D, 3 * D), BF16),
            pltpu.VMEM((D, 3 * D), BF16),
            pltpu.VMEM((D, D), BF16),
            pltpu.VMEM((D, D), BF16),
            pltpu.VMEM((5, 5, KP, 128), F32),
            pltpu.VMEM((D, KP), I32),
            pltpu.VMEM((3 * D // 2, KP), I32),
            pltpu.VMEM((D // 2, KP), I32),
            pltpu.VMEM((D // 2, KP), I32),
            pltpu.VMEM((D, S), F32),
            pltpu.VMEM((5, D, 128), F32),
            pltpu.VMEM((D, 128), F32),
            pltpu.VMEM((NB, 3 * DH, 128 + 2 * HALO, 128), F32),
            pltpu.VMEM((KP // 2, S), I32),
            pltpu.VMEM((KP // 2, S), I32),
            pltpu.VMEM((S, 2 * D), BF16),
            pltpu.VMEM((8, 128), F32),
            pltpu.SemaphoreType.DMA((8,)),
        ],
        compiler_params=pltpu.CompilerParams(
            dimension_semantics=("arbitrary",),
            vmem_limit_bytes=100 * 1024 * 1024),
    )(xa, A_wqkv, A_wo, xb, B_wqkv, B_wo)
    return out.reshape(1, S, 2 * D)
```

```python
import functools
import math

import jax
import jax.numpy as jnp
from jax import lax
import jax.experimental.pallas as pl
import jax.experimental.pallas.tpu as pltpu

S = 2048
D = 576
H = 32
DH = 18
KP = 640
BLK = 512
NB = S // BLK
HALO = 16
WIN = 8
ATT_R = 8
QK_STEP = 3
PV_STEP = 6
WAIT_ROW = 256
PRO_ROW = 304
AT_OT = (7, 9, 10, 12, 15, 17)
F32 = jnp.float32
BF16 = jnp.bfloat16
I32 = jnp.int32
LOG2E = math.log2(math.e)
CSC = (DH ** -0.5) * LOG2E
NEG = -1e9 * LOG2E
ROWS = [(0, 144), (112, 272), (240, 400), (368, 528), (496, 576)]


def _phi(t):
    return jnp.where(t > 0, t + 1.0, jnp.exp(t)) + 1e-6


def _dot(a, b):
    return jnp.dot(a, b, preferred_element_type=F32)


def _dot_nt(a, b):
    return lax.dot_general(a, b, (((1,), (1,)), ((), ())), preferred_element_type=F32)


def _pk(x):
    return pltpu.bitcast(x, I32)


def _upk(x):
    return pltpu.bitcast(x, BF16)


def _token(vals):
    acc = None
    for v in vals:
        b = pltpu.bitcast(v, I32)
        for r in range(0, b.shape[0], 8):
            for c in range(0, b.shape[1], 128):
                x = b[r:r + 8, c:c + 128]
                acc = x if acc is None else acc | x
    return lax.shift_right_logical(lax.shift_right_logical(acc, 31), 1)


def _mark(r, t):
    b, row = divmod(t - 576, 576)
    row = (row // 8) * 8
    return _token([r[row:row + 8, 128 * b:128 * b + 128]])


def _or_f32(x, tok):
    if tok is None:
        return x
    return pltpu.bitcast(pltpu.bitcast(x, I32) | tok, F32)


def _ktile(w_ref, c, col0, ncol):
    if c < 4:
        return w_ref[pl.ds(128 * c, 128), pl.ds(col0, ncol)]
    blk = w_ref[pl.ds(512, 64), pl.ds(col0, ncol)]
    return jnp.concatenate([blk, jnp.zeros_like(blk)], axis=0)


def _kernel(xa_hbm, wa_hbm, woa_hbm, xb_hbm, wb_hbm, wob_hbm, out_hbm,
            xa, xb, wa, wb, woa, wob,
            wt32, wqkT, wbT, woT, mT, pq, T, zb, att, oT, scT, outbuf, mk,
            sem):
    def rows_copy(src, dst, r0, n, col0, ncol, s):
        return pltpu.make_async_copy(src.at[pl.ds(r0, n), pl.ds(col0, ncol)],
                                     dst.at[pl.ds(r0, n), pl.ds(col0, ncol)], sem.at[s])

    def in_copy(name):
        if name == 'w4':
            return rows_copy(wa_hbm, wa, 512, 64, 512, 640, 0)
        if name == 'x4':
            return rows_copy(xa_hbm, xa, 512, 64, 0, BLK, 1)
        if name == 'w0':
            return rows_copy(wa_hbm, wa, 0, 128, 512, 640, 2)
        if name == 'x0':
            return rows_copy(xa_hbm, xa, 0, 128, 0, BLK, 3)
        if name == 'w1':
            return rows_copy(wa_hbm, wa, 128, 128, 512, 640, 4)
        if name == 'x1':
            return rows_copy(xa_hbm, xa, 128, 128, 0, BLK, 5)
        if name == 'w23':
            return rows_copy(wa_hbm, wa, 256, 256, 512, 640, 6)
        if name == 'x23':
            return rows_copy(xa_hbm, xa, 256, 256, 0, BLK, 7)
        if name == 'xa1':
            return rows_copy(xa_hbm, xa, 0, D, BLK, BLK, 0)
        if name == 'wa_q':
            return rows_copy(wa_hbm, wa, 0, D, 0, 512, 1)
        if name == 'xa23':
            return rows_copy(xa_hbm, xa, 0, D, 2 * BLK, 2 * BLK, 2)
        if name == 'wb':
            return pltpu.make_async_copy(wb_hbm, wb, sem.at[3])
        if name == 'wob':
            return pltpu.make_async_copy(wob_hbm, wob, sem.at[4])
        if name == 'wa_v':
            return rows_copy(wa_hbm, wa, 0, D, 1152, 576, 5)
        if name == 'woa':
            return pltpu.make_async_copy(woa_hbm, woa, sem.at[6])
        return pltpu.make_async_copy(xb_hbm, xb.at[pl.ds(0, D), :], sem.at[7])

    outs_started = []

    def out_start(row0, nrow, col0, ncol):
        cp = pltpu.make_async_copy(
            outbuf.at[pl.ds(row0, nrow), pl.ds(col0, ncol)],
            out_hbm.at[pl.ds(row0, nrow), pl.ds(col0, ncol)],
            sem.at[len(outs_started)])
        outs_started.append(cp)
        cp.start()

    queue = []
    due = {}

    def add_due(n, tok):
        due[n] = tok if n not in due else due[n] | tok

    def tile(ref, c, col, n, at, packed):
        if n in at and queue:
            add_due(n, queue.pop(0)())
        tok = due.pop(n, None)
        if packed:
            t = ref[pl.ds(64 * c, 64), pl.ds(col, 128)]
            if tok is not None:
                t = jnp.concatenate([t[0:8, :] | tok, t[8:, :]], axis=0)
            return _upk(t)
        t = ref[pl.ds(128 * c, 128), pl.ds(col, 128)]
        if tok is not None:
            t = jnp.concatenate([_upk(_pk(t[0:16, :]) | tok), t[16:, :]], axis=0)
        return t

    def rhs(ref, col0, at=(), packed=False, bs=range(4)):
        cols = []
        for b in bs:
            tiles = [tile(ref, c, col0 + 128 * b, 5 * b + c, at, packed) for c in range(5)]
            cols.append(jnp.concatenate(tiles, axis=0))
        assert bs[-1] < 3 or not due
        return jnp.concatenate(cols, axis=1)

    def flush():
        while queue:
            queue.pop(0)()

    def lhs(ref, row0):
        return _upk(ref[pl.ds(row0 // 2, D // 2), :])

    def prep_piece(buf, w_ref, col0, ncol, off, dst, base, c):
        def run():
            wt32[buf, c, pl.ds(0, ncol), :] = _ktile(w_ref, c, col0, ncol).T.astype(F32)
            outs = []
            for d in range(0, DH, 2):
                r0 = wt32[buf, c, pl.ds(off + d, 32, stride=DH), :]
                r1 = wt32[buf, c, pl.ds(off + d + 1, 32, stride=DH), :]
                v = _pk(jnp.concatenate([r0, r1], axis=0).astype(BF16))
                dst[pl.ds(base // 2 + 16 * d, 32), pl.ds(128 * c, 128)] = v
                outs.append(v)
            return _token(outs)
        return run

    def perm_t_piece(buf, dst, c):
        nrow = 128 if c < 4 else 64
        outs = []
        for kt in range(5):
            ds_ = range(4 * kt, min(4 * kt + 4, DH))
            rows = [wt32[buf, c, pl.ds(d, 32, stride=DH), :] for d in ds_]
            if kt == 4:
                rows.append(jnp.zeros((64, 128), F32))
            tile = _pk(jnp.concatenate(rows, axis=0).astype(BF16).T[:nrow, :])
            dst[pl.ds(64 * c, nrow // 2), pl.ds(128 * kt, 128)] = tile
            outs.append(tile)
        return _token(outs)

    def prep_wo_piece(buf, c):
        def run():
            if c < 4:
                wt32[buf, c, pl.ds(0, D), :] = wob[:, pl.ds(128 * c, 128)].astype(F32)
            else:
                wt32[buf, 4, pl.ds(0, D), :] = jnp.concatenate(
                    [wob[:, pl.ds(512, 64)].astype(F32), jnp.zeros((D, 64), F32)], axis=1)
            return perm_t_piece(buf, woT, c)
        return run

    def a_kt(i, at_k=(), at_t=(), kT=None, waits=()):
        if kT is None:
            kT = _dot(lhs(wqkT, D), rhs(xa, i * BLK, at_k))
        pk = _phi(kT).astype(BF16)
        for c in range(5):
            xrow = jnp.concatenate(
                [tile(xa, c, i * BLK + 128 * b, 4 * c + b, at_t, False) for b in range(4)], axis=1)
            t = _dot_nt(pk, xrow)
            if i == 0:
                T[c] = t
            else:
                T[c] += t
        assert not due

    def a_q(i, at=()):
        qT = _dot(lhs(wqkT, 0), rhs(xa, i * BLK, at))
        pq[:, pl.ds(i * BLK, BLK)] = _phi(qT)
        return qT

    def b_part(j, p, at=()):
        first = j == 0
        lane = lax.broadcasted_iota(I32, (HALO, 128), 1)
        r32 = _dot(lhs(wbT, D * p), rhs(xb, j * BLK, at))
        r = r32.astype(BF16)
        for d in range(DH):
            tl = jnp.concatenate(
                [r[32 * d:32 * d + 32, 128 * b:128 * b + 128] for b in range(4)], axis=0)
            tt = tl.T.astype(F32)
            att[j, p * DH + d, pl.ds(HALO, 128), :] = tt
            tvals = [tt[120:128, :]]
            if p > 0:
                cur = pltpu.roll(tt[128 - HALO:, :], 32, 1)
                if first:
                    if p == 1:
                        prev = jnp.zeros((HALO, 128), F32)
                    else:
                        prev = jnp.broadcast_to(tt[0:1, :], (HALO, 128))
                else:
                    prev = att[j - 1, p * DH + d, pl.ds(128 + HALO, HALO), :]
                halo = jnp.where(lane < 32, prev, cur)
                att[j, p * DH + d, pl.ds(0, HALO), :] = halo
                tvals.append(halo)
                if j < NB - 1:
                    att[j, p * DH + d, pl.ds(128 + HALO, HALO), :] = cur
            add_due(4 + (d * 12) // DH, _token(tvals))
        return r32

    def att_group(j, g):
        R = ATT_R
        base = HALO + g * R
        ls = [None] * WIN
        csc = None
        for d in range(DH):
            if d % QK_STEP == 0:
                tok = yield
                csc = _or_f32(jnp.full((R, 128), CSC, F32), tok)
            q = att[j, d, pl.ds(base, R), :] * csc
            for w in range(WIN):
                t = q * att[j, DH + d, pl.ds(base - 2 * w, R), :]
                ls[w] = t if ls[w] is None else ls[w] + t
        if g * R < HALO and j == 0:
            pos = (lax.broadcasted_iota(I32, (R, 128), 0) + g * R
                   + (lax.broadcasted_iota(I32, (R, 128), 1) // 32) * 128)
            ls = [ls[0]] + [jnp.where(pos >= 2 * w, ls[w], NEG) for w in range(1, WIN)]
        m = functools.reduce(jnp.maximum, ls)
        es = [jnp.exp2(l - m) for l in ls]
        inv = 1.0 / functools.reduce(lambda a, b: a + b, es)
        ps = None
        for d in range(DH):
            if d % PV_STEP == 0:
                tok = yield
                invt = _or_f32(inv, tok)
                ps = [e * invt for e in es]
            acc = None
            for w in range(WIN):
                t = ps[w] * att[j, 2 * DH + d, pl.ds(base - 2 * w, R), :]
                acc = t if acc is None else acc + t
            att[j, d, pl.ds(base, R), :] = acc

    NPIECE = (128 // ATT_R) * (DH // QK_STEP + DH // PV_STEP)
    state = {'gens': [], 'left': 0}

    def att_begin(j):
        gens = [att_group(j, g) for g in range(128 // ATT_R)]
        for gen in gens:
            next(gen)
        state['gens'] = gens
        state['left'] = NPIECE

    def release(r, n):
        n = min(n, state['left'])
        for i in range(n):
            tok = _mark(r, 576 + (2304 * i) // n)
            gen = state['gens'][0]
            try:
                gen.send(tok)
            except StopIteration:
                state['gens'].pop(0)
            state['left'] -= 1

    def ot_piece(j, d0, d1):
        def run():
            outs = []
            for d in range(d0, d1):
                ot = _pk(att[j, d, pl.ds(HALO, 128), :].astype(BF16).T)
                for b in range(4):
                    oT[pl.ds(16 * d, 16), pl.ds(j * BLK + 128 * b, 128)] = ot[16 * b:16 * b + 16, :]
                outs.append(ot[56:64, :])
            return _token(outs)
        return run

    def a_scale(j):
        for b in range(4):
            col = pl.ds(j * BLK + 128 * b, 128)
            den = None
            for d in range(DH):
                t = pq[pl.ds(32 * d, 32), col] * zb[pl.ds(32 * d, 32), :]
                den = t if den is None else den + t
            inv = 1.0 / (den + 1e-6)
            for d in range(DH):
                scT[pl.ds(16 * d, 16), col] = _pk((pq[pl.ds(32 * d, 32), col] * inv).astype(BF16))

    def out_b(j):
        return _dot(lhs(woT, 0), rhs(oT, j * BLK, packed=True))

    def out_a(j, at=()):
        return _dot(lhs(mT, 0), rhs(scT, j * BLK, at, packed=True))

    def store_t(row0, col0, blk):
        bt = blk.T
        outbuf[pl.ds(row0, 128), pl.ds(col0, blk.shape[0])] = bt
        return _token([bt[112:128, :]])

    def store_part(j, kind, oa, ob, n0, dn):
        for b in range(4):
            cs = slice(128 * b, 128 * b + 128)
            rows = []
            if 'a' in kind:
                rows.append(oa[0:512, cs])
            if 'm' in kind:
                rows += [oa[512:D, cs], ob[0:192, cs]]
            if 'b' in kind:
                rows.append(ob[192:D, cs])
            col0 = {'a': 0, 'm': 512, 'b': 768}[kind[0]]
            add_due(n0 + dn * b, store_t(j * BLK + 128 * b, col0, jnp.concatenate(rows, axis=0)))

    def a_small_g():
        kvs = []
        for jt, (r0, r1) in enumerate(ROWS):
            n = r1 - r0
            w = 128 if jt < 4 else 64
            tb = jnp.concatenate([T[c, pl.ds(r0, n), :] for c in range(5)], axis=1)[:, :D].astype(BF16)
            g = _dot(tb, wa[:, pl.ds(1152 + 128 * jt, w)])
            rh = (lax.broadcasted_iota(I32, (n, w), 0) + r0) // DH
            ch = (lax.broadcasted_iota(I32, (n, w), 1) + 128 * jt) // DH
            kvs.append(jnp.where(rh == ch, g, 0.0).astype(BF16))
        lane = lax.broadcasted_iota(I32, (32, 128), 1)
        for d in range(DH):
            t = T[4, pl.ds(d, 32, stride=DH), :]
            zb[pl.ds(32 * d, 32), :] = jnp.where(lane >= 64, t, pltpu.roll(t, 64, 1))
        return kvs

    def a_small_m(buf, kvs):
        for c in range(5):
            wt32[buf, c, pl.ds(0, D), :] = jnp.zeros((D, 128), F32)
        for jt, (r0, r1) in enumerate(ROWS):
            n = r1 - r0
            if jt < 4:
                mrow = _dot(kvs[jt], woa[pl.ds(128 * jt, 128), :])
            else:
                w4 = woa[pl.ds(512, 64), :]
                mrow = jnp.concatenate([
                    _dot(kvs[4], w4[:, :384]),
                    jnp.concatenate([_dot(kvs[4][:48], w4[:, 384:]), _dot(kvs[4][48:], w4[:, 384:])], axis=0)],
                    axis=1)
            for c in range(4):
                wt32[buf, c, pl.ds(r0, n), :] += mrow[:, 128 * c:128 * c + 128]
            wt32[buf, 4, pl.ds(r0, n), pl.ds(0, 64)] += mrow[:, 512:576]

    for name in ('w4', 'x4', 'w0', 'x0', 'w1', 'x1', 'w23', 'x23'):
        in_copy(name).start()
    xa[pl.ds(D, KP - D), :] = jnp.ones((KP - D, S), BF16)
    xb[pl.ds(D, KP - D), :] = jnp.zeros((KP - D, S), BF16)
    oT[pl.ds(D // 2, (KP - D) // 2), :] = jnp.zeros(((KP - D) // 2, S), I32)
    scT[pl.ds(D // 2, (KP - D) // 2), :] = jnp.zeros(((KP - D) // 2, S), I32)

    def wk_t(c):
        wqkT[pl.ds(D // 2, D // 2), pl.ds(128 * c, 128)] = _pk(_ktile(wa, c, 512, 640).T[64:, :])

    def kt_part(c0, nc):
        return _dot(_upk(wqkT[pl.ds(D // 2, D // 2), pl.ds(128 * c0, 128 * nc)]),
                    xa[pl.ds(128 * c0, 128 * nc), pl.ds(0, BLK)])

    in_copy('w4').wait()
    wk_t(4)
    kT = None
    for c, ws, nxt, tr in [
            (4, ('x4', 'w0'), (), (0,)),
            (0, ('x0', 'w1'), (), (1,)),
            (1, ('x1', 'w23'), ('xa1', 'wa_q'), (2, 3))]:
        for name in ws:
            in_copy(name).wait()
        for name in nxt:
            in_copy(name).start()
        part = kt_part(c, 1)
        for t in tr:
            wk_t(t)
        mk[...] = part[0:8, 0:128]
        kT = part if kT is None else kT + part
    in_copy('x23').wait()
    in_copy('xa23').start()
    in_copy('wb').start()
    a_kt(0, kT=kT + kt_part(2, 2))

    in_copy('xa1').wait()
    in_copy('wa_q').wait()
    for name in ('wob', 'wa_v', 'woa', 'xb'):
        in_copy(name).start()
    for c in range(5):
        queue.append(prep_piece(3, wa, 0, 640, 0, wqkT, 0, c))
    AT5 = (5, 8, 11, 14, 17)
    a_kt(1, (9, 14, 19), (4, 9))

    in_copy('xa23').wait()
    in_copy('wb').wait()
    for c in range(5):
        queue.append(prep_piece(0, wb, 0, 640, 0, wbT, 0, c))
    for c in range(5):
        queue.append(prep_piece(1, wb, 512, 640, 64, wbT, D, c))
    for c in range(5):
        queue.append(prep_piece(2, wb, 1152, 576, 0, wbT, 2 * D, c))
    a_kt(2, (6, 11, 16), (1, 6, 11, 16))
    a_kt(3, (1, 6, 11, 16), (1, 6, 11, 16))
    assert not queue

    for name in ('wob', 'wa_v', 'woa', 'xb'):
        in_copy(name).wait()
    kvs = a_small_g()
    for c in range(5):
        queue.append(prep_wo_piece(4, c))
    b_part(0, 0, AT5)
    a_small_m(0, kvs)
    b_part(0, 1)
    for c in range(5):
        queue.append(functools.partial(perm_t_piece, 0, mT, c))
    b_part(0, 2, AT5)

    def spread(rs):
        for i, (fn, wgt) in enumerate(rs):
            tot = sum(w for _, w in rs[i:])
            n = int(round(state['left'] * wgt / tot))
            release(fn(), n)
        assert state['left'] == 0

    def queue_ot(j):
        for d0 in range(0, DH, 3):
            queue.append(ot_piece(j, d0, d0 + 3))

    res = {}

    def keep(name, fn):
        def run():
            res[name] = fn()
            return res[name]
        return run

    def bf(name):
        return res[name].astype(BF16)

    def job(name, fn, pre=None):
        def run():
            if pre is not None:
                pre()
            res[name] = fn()
            return res[name]
        return run

    def out_block(j):
        out_start(j * BLK, BLK, 0, 2 * D)

    att_begin(0)
    spread([(lambda: b_part(1, 0), 1), (lambda: b_part(1, 1), 1), (lambda: b_part(1, 2), 1),
            (lambda: a_q(0), 1)])
    a_scale(0)
    queue_ot(0)
    att_begin(1)
    spread([(job('oa0', lambda: out_a(0, AT_OT)), 0.5),
            (job('ob0', lambda: out_b(0), lambda: store_part(0, 'a', bf('oa0'), None, 4, 4)), 1),
            (job('x', lambda: b_part(2, 0),
                 lambda: (store_part(0, 'mb', bf('oa0'), bf('ob0'), 4, 4), out_block(0))), 1),
            (lambda: b_part(2, 1), 1), (lambda: b_part(2, 2), 1)])
    queue_ot(1)
    att_begin(2)
    spread([(lambda: a_q(1, AT_OT), 0.5),
            (job('ob1', lambda: out_b(1)), 1),
            (job('x', lambda: b_part(3, 0),
                 lambda: (store_part(1, 'b', None, bf('ob1'), 4, 4), a_scale(1))), 1),
            (lambda: b_part(3, 1), 1), (lambda: b_part(3, 2), 1)])
    queue_ot(2)
    att_begin(3)
    spread([(job('oa1', lambda: out_a(1, AT_OT)), 0.5),
            (job('ob2', lambda: out_b(2),
                 lambda: (store_part(1, 'am', bf('oa1'), bf('ob1'), 4, 4), out_block(1))), 1),
            (job('x', lambda: a_q(2), lambda: store_part(2, 'b', None, bf('ob2'), 4, 4)), 1),
            (job('oa2', lambda: out_a(2), lambda: a_scale(2)), 1),
            (job('x', lambda: a_q(3),
                 lambda: (store_part(2, 'am', bf('oa2'), bf('ob2'), 4, 4), out_block(2))), 1)])
    a_scale(3)
    oa = out_a(3).astype(BF16)
    for d0 in range(0, DH, 3):
        ot_piece(3, d0, d0 + 3)()
    j = NB - 1
    store_part(j, 'a', oa, None, 4, 2)
    out_start(j * BLK, BLK, 0, 512)
    lw = woT[...]
    for b in range(4):
        if b == 3:
            lw = jnp.concatenate([
                lw[:, :512],
                jnp.concatenate([lw[:208, 512:], lw[208:216, 512:] | last_tok, lw[216:, 512:]], axis=0)], axis=1)
        ob = _dot(_upk(lw), rhs(oT, j * BLK, packed=True, bs=[b])).astype(BF16)
        blk = jnp.concatenate([oa[512:D, 128 * b:128 * b + 128], ob], axis=0)
        row0 = j * BLK + 128 * b
        if b < 3:
            tok = store_t(row0, 512, blk)
            if b < 2:
                add_due(13 + 4 * b, tok)
            else:
                last_tok = tok
            if b == 1:
                out_start(j * BLK, 256, 512, 640)
            if b == 2:
                out_start(row0, 128, 512, 640)
        else:
            store_t(row0, 512, blk[:512])
            out_start(row0, 128, 512, 512)
            store_t(row0, 1024, blk[512:])
            out_start(row0, 128, 1024, 128)
    for cp in outs_started:
        cp.wait()


@jax.jit
def pallas_concat_heads__linear_attn_block__sliding_local_dilated__prompt_kernel(A_x, A_wqkv, A_wo, B_x, B_wqkv, B_wo):
    xa = jnp.transpose(A_x[0])
    xb = jnp.transpose(B_x[0])
    anyspec = pl.BlockSpec(memory_space=pl.ANY)
    out = pl.pallas_call(
        _kernel,
        grid=(1,),
        in_specs=[anyspec] * 6,
        out_specs=anyspec,
        out_shape=jax.ShapeDtypeStruct((S, 2 * D), BF16),
        scratch_shapes=[
            pltpu.VMEM((KP, S), BF16),
            pltpu.VMEM((KP, S), BF16),
            pltpu.VMEM((D, 3 * D), BF16),
            pltpu.VMEM((D, 3 * D), BF16),
            pltpu.VMEM((D, D), BF16),
            pltpu.VMEM((D, D), BF16),
            pltpu.VMEM((5, 5, KP, 128), F32),
            pltpu.VMEM((D, KP), I32),
            pltpu.VMEM((3 * D // 2, KP), I32),
            pltpu.VMEM((D // 2, KP), I32),
            pltpu.VMEM((D // 2, KP), I32),
            pltpu.VMEM((D, S), F32),
            pltpu.VMEM((5, D, 128), F32),
            pltpu.VMEM((D, 128), F32),
            pltpu.VMEM((NB, 3 * DH, 128 + 2 * HALO, 128), F32),
            pltpu.VMEM((KP // 2, S), I32),
            pltpu.VMEM((KP // 2, S), I32),
            pltpu.VMEM((S, 2 * D), BF16),
            pltpu.VMEM((8, 128), F32),
            pltpu.SemaphoreType.DMA((8,)),
        ],
        compiler_params=pltpu.CompilerParams(
            dimension_semantics=("arbitrary",),
            vmem_limit_bytes=100 * 1024 * 1024),
    )(xa, A_wqkv, A_wo, xb, B_wqkv, B_wo)
    return out.reshape(1, S, 2 * D)
```

```python
import functools
import math

import jax
import jax.numpy as jnp
from jax import lax
import jax.experimental.pallas as pl
import jax.experimental.pallas.tpu as pltpu

S = 2048
D = 576
H = 32
DH = 18
KP = 640
HM = D // 2
BLK = 512
NB = S // BLK
HALO = 16
WIN = 8
ATT_R = 8
QK_STEP = 3
PV_STEP = 6
F32 = jnp.float32
BF16 = jnp.bfloat16
I32 = jnp.int32
LOG2E = math.log2(math.e)
CSC = (DH ** -0.5) * LOG2E
NEG = -1e9 * LOG2E
ROWS = [(0, 144), (112, 272), (240, 400), (368, 528), (496, 576)]

LB = dict(I1=0, I2=1, a1=2, a2=3, b1=4, b2=5, c1=6, c2=7, d1=8, d2=9,
          p11_1=10, p11_2=11, p22_1=12, p22_2=13, p12=14, p21=15)
PAT = {
    'I': ('I1', ('I1', 'I2'), ((0, 1), (3, 1))),
    'a': ('a1', ('a1', 'a2'), ((2, 1), (3, -1))),
    'b': ('b1', ('b1', 'b2'), ((1, 1), (3, 1))),
    'c': ('c1', ('c1', 'c2'), ((0, 1), (2, 1))),
    'd': ('d1', ('d1', 'd2'), ((0, -1), (1, 1))),
    '11': ('p11_1', ('p11_1', 'p11_2'), ((0, 1),)),
    '22': ('p22_1', ('p22_1', 'p22_2'), ((3, 1),)),
    '12': ('p12', ('p12',), ((1, 1),)),
    '21': ('p21', ('p21',), ((2, 1),)),
    'X': ('I2', ('X',), ((1, 1), (2, 1))),
}
SEQ = {
    0: ('I', 'a', 'b', '22', 'c', '11', 'd', '21', 'X', '12'),
    1: ('21', 'a', 'I', 'c', 'b', '22', 'X', '12', 'd', '11'),
    2: ('I', 'a', 'b', '22', 'c', '21', 'X', 'd', '12', '11'),
    3: ('21', 'a', 'c', 'X', '12', 'b', 'I', '22', 'd', '11'),
    'cold': ('a', 'd', 'I', 'b', '22', 'c', '11', '21', 'X', '12'),
}
PKOP = dict(o11=0, o21=1, c1=2, o12=3, o22=4, c2=5, sd=6, sx=7, m2=8, m1=9)
TP = (('p11_1', 'o11'), ('c1', 'c1'), ('p11_2', 'o11'), ('c2', 'c1'), ('p21', 'o21'),
      ('p22_1', 'o22'), ('a1', 'm2'), ('a2', 'm2'), ('d1', 'm1'), ('d2', 'm1'), ('I1', 'sd'),
      ('b1', 'c2'), ('p22_2', 'o22'), ('p12', 'o12'), ('b2', 'c2'), ('E', 'sd'), ('E', 'sx'))
TIDX = {t: i for i, t in enumerate(TP)}


def _phi(t):
    return jnp.where(t > 0, t + 1.0, jnp.exp(t)) + 1e-6


def _dot(a, b):
    return jnp.dot(a, b, preferred_element_type=F32)


def _dot_nt(a, b):
    return lax.dot_general(a, b, (((1,), (1,)), ((), ())), preferred_element_type=F32)


def _pk(x):
    return pltpu.bitcast(x, I32)


def _upk(x):
    return pltpu.bitcast(x, BF16)


def _pkf(x):
    return _pk(x.astype(BF16))


def _ipk(a, b):
    return pltpu.bitcast(pltpu.pack_elementwise([a, b], packed_dtype=BF16), I32)


def _pki(x):
    out = [_ipk(x[r:r + 8], x[r + 8:r + 16]) for r in range(0, x.shape[0], 16)]
    return out[0] if len(out) == 1 else jnp.concatenate(out, axis=0)


def _par(p, s):
    return pltpu.unpack_elementwise(pltpu.bitcast(p, jnp.uint32), index=s,
                                    packed_dtype=BF16, unpacked_dtype=F32)


class _EO:
    def __init__(self, e, o):
        self.e, self.o = e, o

    def __add__(self, y):
        return _EO(self.e + y.e, self.o + y.o)

    def __sub__(self, y):
        return _EO(self.e - y.e, self.o - y.o)

    def __mul__(self, c):
        return _EO(self.e * c, self.o * c)

    def pack(self):
        return _ipk(self.e, self.o)

    def pack_split(self):
        return _pkf(jnp.concatenate([self.e, self.o], axis=0))


def _eo(p):
    return _EO(_par(p, 0), _par(p, 1))


def _token(vals):
    acc = None
    for v in vals:
        b = pltpu.bitcast(v, I32)
        for r in range(0, b.shape[0], 8):
            for c in range(0, b.shape[1], 128):
                x = b[r:r + 8, c:c + 128]
                acc = x if acc is None else acc | x
    return lax.shift_right_logical(lax.shift_right_logical(acc, 31), 1)


def _or_f32(x, tok):
    if tok is None:
        return x
    return pltpu.bitcast(pltpu.bitcast(x, I32) | tok, F32)


def _ktile(w_ref, c, col0, ncol):
    if c < 4:
        return w_ref[pl.ds(128 * c, 128), pl.ds(col0, ncol)]
    blk = w_ref[pl.ds(512, 64), pl.ds(col0, ncol)]
    return jnp.concatenate([blk, blk], axis=0)


def _kernel(xa_hbm, wa_hbm, woa_hbm, xb_hbm, wb_hbm, wob_hbm, out_hbm,
            xa, xb, wa, wb, woa, wob,
            wt32, wpl, L, xca, xcb, pkc, TA, pq, T, zacc, zb, att, oT, oc, scT, scc, outbuf, mk,
            sem):
    def rows_copy(src, dst, r0, n, col0, ncol, s):
        return pltpu.make_async_copy(src.at[pl.ds(r0, n), pl.ds(col0, ncol)],
                                     dst.at[pl.ds(r0, n), pl.ds(col0, ncol)], sem.at[s])

    def in_copy(name):
        if name == 'w4':
            return rows_copy(wa_hbm, wa, 512, 64, 512, 640, 0)
        if name == 'x4':
            return rows_copy(xa_hbm, xa, 512, 64, 0, BLK, 1)
        if name == 'w0':
            return rows_copy(wa_hbm, wa, 0, 128, 512, 640, 2)
        if name == 'x0':
            return rows_copy(xa_hbm, xa, 0, 128, 0, BLK, 3)
        if name == 'w1':
            return rows_copy(wa_hbm, wa, 128, 128, 512, 640, 4)
        if name == 'x1':
            return rows_copy(xa_hbm, xa, 128, 128, 0, BLK, 5)
        if name == 'w23':
            return rows_copy(wa_hbm, wa, 256, 256, 512, 640, 6)
        if name == 'x23':
            return rows_copy(xa_hbm, xa, 256, 256, 0, BLK, 7)
        if name == 'xa1':
            return rows_copy(xa_hbm, xa, 0, D, BLK, BLK, 0)
        if name == 'wa_q':
            return rows_copy(wa_hbm, wa, 0, D, 0, 512, 1)
        if name == 'xa23':
            return rows_copy(xa_hbm, xa, 0, D, 2 * BLK, 2 * BLK, 2)
        if name == 'wb':
            return pltpu.make_async_copy(wb_hbm, wb, sem.at[3])
        if name == 'wob':
            return pltpu.make_async_copy(wob_hbm, wob, sem.at[4])
        if name == 'wa_v':
            return rows_copy(wa_hbm, wa, 0, D, 1152, 576, 5)
        if name == 'woa':
            return pltpu.make_async_copy(woa_hbm, woa, sem.at[6])
        return pltpu.make_async_copy(xb_hbm, xb, sem.at[7])

    outs_started = []

    def out_start(row0, nrow, col0, ncol):
        cp = pltpu.make_async_copy(
            outbuf.at[pl.ds(row0, nrow), pl.ds(col0, ncol)],
            out_hbm.at[pl.ds(row0, nrow), pl.ds(col0, ncol)],
            sem.at[len(outs_started)])
        outs_started.append(cp)
        cp.start()

    lo8 = lax.broadcasted_iota(I32, (8, 128), 1) < 64

    def lo(nr):
        return jnp.concatenate([lo8] * (nr // 8), axis=0)

    queue = []
    due = {}
    st = {'tiles': 0, 'slot': 0}

    def add_due(n, tok):
        due[n] = tok if n not in due else due[n] | tok

    def begin_dot():
        st['slot'] = 0

    def end_dot():
        assert not due, due

    def rtile(src, j, n, name, at):
        orig, packed, comb = src
        col = j * BLK

        def X(c, b, r0=0, nr=128):
            if packed:
                return orig[pl.ds(64 * c + r0 // 2, nr // 2), pl.ds(col + 128 * b, 128)]
            return _pk(orig[pl.ds(128 * c + r0, nr), pl.ds(col + 128 * b, 128)])

        def K(g, k, r0=0, nr=128):
            return comb[j, n, g, k, pl.ds(r0 // 2, nr // 2), :]

        n1, n2 = n, n + 2
        parts = {
            'I1': lambda: [K(0, 0)], 'a1': lambda: [X(0, n1)], 'b1': lambda: [K(0, 1)],
            'c1': lambda: [K(0, 2)], 'd1': lambda: [X(1, n2)], 'p22_1': lambda: [K(0, 3)],
            'p11_1': lambda: [K(0, 4)],
            'I2': lambda: [K(1, 0, 0, 64), None], 'X': lambda: [None, K(1, 0, 64, 64)],
            'E': lambda: [K(1, 0)],
            'a2': lambda: [X(2, n1, 0, 64), X(2, n2, 64, 64)],
            'd2': lambda: [X(3, n2, 0, 64), X(3, n1, 64, 64)],
            'b2': lambda: [K(1, 1)], 'c2': lambda: [K(1, 2)],
            'p22_2': lambda: [K(1, 3, 0, 64), X(4, n2, 0, 64)],
            'p11_2': lambda: [K(1, 4, 0, 64), X(4, n1, 0, 64)],
            'p12': lambda: [X(4, n2, 0, 64), K(1, 4, 64, 64)],
            'p21': lambda: [X(4, n1, 0, 64), K(1, 3, 64, 64)],
        }
        s = st['slot']
        if s in at and queue:
            add_due(s, queue.pop(0)())
        tok = due.pop(s, None)
        st['slot'] += 1
        st['tiles'] += 1
        out = []
        for p in parts[name]():
            if p is None:
                p = jnp.zeros((32, 128), I32)
            elif tok is not None:
                p = jnp.concatenate([p[0:8, :] | tok, p[8:, :]], axis=0)
                tok = None
            out.append(p)
        return _upk(out[0] if len(out) == 1 else jnp.concatenate(out, axis=0))

    def half(m, src, j, n, at, marks, cold=False):
        acc = [None] * 4
        for pat in SEQ['cold' if cold else st['tiles'] % 4]:
            lb, rts, outs = PAT[pat]
            lhs = _upk(L[m, :, pl.ds(128 * LB[lb], 128 * len(rts))])
            tiles = [rtile(src, j, n, r, at) for r in rts]
            p = _dot(lhs, tiles[0] if len(tiles) == 1 else jnp.concatenate(tiles, axis=0))
            marks[(st['tiles'] - 1) // 4] = p
            for q, sg in outs:
                if acc[q] is None:
                    acc[q] = (p, sg)
                else:
                    v, s0 = acc[q]
                    if s0 == sg:
                        acc[q] = (v + p, sg)
                    elif s0 > 0:
                        acc[q] = (v - p, 1)
                    else:
                        acc[q] = (p - v, 1)
        assert all(s == 1 for _, s in acc)
        return [v for v, _ in acc]

    def sdot(m, src, j, at=(), cold=False, ns=(0, 1)):
        begin_dot()
        marks = {}
        t0 = st['tiles']
        C = {}
        for n in ns:
            c11, c12, c21, c22 = half(m, src, j, n, at, marks, cold and n == ns[0])
            C[(0, n)], C[(0, n + 2)], C[(1, n)], C[(1, n + 2)] = c11, c12, c21, c22
        end_dot()
        return C, (marks, t0, st['tiles'])

    def mark(mi, f):
        marks, t0, t1 = mi
        pos = (t0 + (t1 - t0) * f) / 4.0
        r = int(pos)
        row = int((pos - r) * HM) // 8 * 8
        return _token([marks[r][row:row + 8, :]])

    def flush():
        while queue:
            queue.pop(0)()

    def emit_l(m, prow, g, a11, a12, a21, a22, a11p, a22p, a13p, a23p, split=False):
        nr = a11.e.shape[0]
        outs = []
        _pkf = _EO.pack_split if split else _EO.pack

        def put(name, v):
            L[m, pl.ds(prow, nr), pl.ds(128 * LB[name], 128)] = v
            outs.append(v)

        pi = _pkf(a11 + a22)
        p11 = _pkf(a12 - a22)
        p22 = _pkf(a21 - a11)
        if g == 0:
            put('I1', pi)
            put('a1', _pkf(a21 + a22))
            put('b1', a11p)
            put('c1', a22p)
            put('d1', _pkf(a11 + a12))
            put('p11_1', p11)
            put('p22_1', p22)
        else:
            m8 = lo(nr)
            sgn = jnp.where(m8, 1.0, -1.0).astype(F32)
            put('I2', pi)
            put('a2', _pkf((a21 + a22) * sgn))
            put('d2', _pkf((a11 + a12) * sgn))
            put('b2', jnp.where(m8, a11p, a22p))
            put('c2', jnp.where(m8, a22p, a11p))
            put('p11_2', jnp.where(m8, p11, a13p))
            put('p22_2', jnp.where(m8, p22, a23p))
            put('p12', jnp.where(m8, a13p, p11))
            put('p21', jnp.where(m8, a23p, p22))
        return outs

    def build_piece(m, pb, r0, r1, split=False):
        def run():
            outs = []
            for r in range(r0, r1, 8):
                def ld(i, c):
                    return wpl[pb, pl.ds(HM // 2 * i + r, 8), pl.ds(128 * c, 128)]
                for g in (0, 1):
                    ps = [ld(0, 2 * g), ld(0, 2 * g + 1), ld(1, 2 * g), ld(1, 2 * g + 1)]
                    fs = [_eo(p) for p in ps]
                    ex = (ld(0, 4), ld(1, 4)) if g else (None, None)
                    if split:
                        ps = [f.pack_split() for f in fs]
                        ex = [_eo(e).pack_split() if g else None for e in ex]
                    outs += emit_l(m, r, g, *fs, ps[0], ps[3], *ex, split=split)
            return _token(outs)
        return run

    def tr_piece(buf, w_ref, col0, ncol, c):
        def run():
            t = _ktile(w_ref, c, col0, ncol).T.astype(F32)
            wt32[buf, c, pl.ds(0, ncol), :] = t
            return _token([t[r:r + 8, :] for r in range(120, ncol, 128)] + [t[ncol - 8:, :]])
        return run

    def comb_piece(buf, m, off, g, d0, d1):
        def run():
            outs = []
            for d in range(d0, d1):
                def ld(i, c):
                    return _EO(*[wt32[buf, c, pl.ds(off + d + 9 * i + DH * s, 16, stride=2 * DH), :]
                                 for s in (0, 1)])
                fs = [ld(0, 2 * g), ld(0, 2 * g + 1), ld(1, 2 * g), ld(1, 2 * g + 1)]
                ex = (ld(0, 4).pack(), ld(1, 4).pack()) if g else (None, None)
                outs += emit_l(m, 16 * d, g, *fs, fs[0].pack(), fs[3].pack(), *ex)
            return _token(outs)
        return run

    def queue_prep(buf, w_ref, col0, ncol, off, m):
        queue.append(tr_piece(buf, w_ref, col0, ncol, 0))
        queue.append(tr_piece(buf, w_ref, col0, ncol, 1))
        queue.append(comb_piece(buf, m, off, 0, 0, 5))
        queue.append(tr_piece(buf, w_ref, col0, ncol, 2))
        queue.append(comb_piece(buf, m, off, 0, 5, 9))
        queue.append(tr_piece(buf, w_ref, col0, ncol, 3))
        queue.append(tr_piece(buf, w_ref, col0, ncol, 4))
        for d0 in (0, 3, 6):
            queue.append(comb_piece(buf, m, off, 1, d0, d0 + 3))

    def perm_t_piece(buf, pb, c):
        nrow = 128 if c < 4 else 64
        outs = []
        for kt in range(5):
            ds_ = range(4 * kt, 4 * kt + 4) if kt < 4 else (16, 17, 16, 17)
            rows = [wt32[buf, c, pl.ds(d, 32, stride=DH), :] for d in ds_]
            tile = _pk(_upk(_pki(jnp.concatenate(rows, axis=0))).T[:nrow, :])
            wpl[pb, pl.ds(64 * c, nrow // 2), pl.ds(128 * kt, 128)] = tile
            outs.append(tile)
        return _token(outs)

    def prep_wo_piece(buf, c):
        def run():
            if c < 4:
                wt32[buf, c, pl.ds(0, D), :] = wob[:, pl.ds(128 * c, 128)].astype(F32)
            else:
                wt32[buf, 4, pl.ds(0, D), :] = jnp.concatenate(
                    [wob[:, pl.ds(512, 64)].astype(F32), jnp.zeros((D, 64), F32)], axis=1)
            return perm_t_piece(buf, 1, c)
        return run

    def emit_r(comb, j, n, g, r, b11, b12, b21, b22):
        hi = g == 1 and r >= 64
        vals = [b12 + b21 if hi else b11 + b22,
                b22 - b12 if hi else b12 - b22,
                b11 - b21 if hi else b21 - b11,
                b11 + b12, b21 + b22]
        outs = []
        for k, v in enumerate(vals):
            v = v.pack() if isinstance(v, _EO) else _pki(v)
            comb[j, n, g, k, pl.ds(r // 2, v.shape[0]), :] = v
            outs.append(v)
        return outs

    def xc_piece(x_ref, comb, j, n, g):
        def run():
            outs = []
            for r in range(0, 128, 16):
                def ld(c, b):
                    return _eo(_pk(x_ref[pl.ds(128 * c + r, 16), pl.ds(j * BLK + 128 * b, 128)]))
                outs += emit_r(comb, j, n, g, r,
                               ld(2 * g, n), ld(2 * g, n + 2), ld(2 * g + 1, n), ld(2 * g + 1, n + 2))
            return _token(outs)
        return run

    def queue_xc(x_ref, comb, j):
        for n in (0, 1):
            for g in (0, 1):
                queue.append(xc_piece(x_ref, comb, j, n, g))

    SXA = (xa, False, xca)
    SXB = (xb, False, xcb)
    SO = (oT, True, oc)
    SSC = (scT, True, scc)

    def pk_ops(i, C, ns=(0, 1)):
        for n in ns:
            a11, a12, a21, a22 = [_phi(C[q]) for q in ((0, n), (0, n + 2), (1, n), (1, n + 2))]
            ops = dict(o11=a11, o21=a21, c1=a11 + a21, o12=a12, o22=a22, c2=a12 + a22,
                       sd=a11 + a22, sx=a12 + a21, m2=a21 - a22, m1=a12 - a11)
            for name, v in ops.items():
                pkc[PKOP[name], :, pl.ds(128 * (2 * i + n), 128)] = _pki(v)
            for hf, v in enumerate((a11 + a12, a21 + a22)):
                if i == 0 and n == 0:
                    zacc[pl.ds(HM * hf, HM), :] = v
                else:
                    zacc[pl.ds(HM * hf, HM), :] += v

    def tdot(k0, nk, at=(), split_last=False):
        begin_dot()
        for t, (rname, op) in enumerate(TP):
            lhs = _upk(pkc[PKOP[op], :, pl.ds(128 * k0, 128 * nk)])
            tiles = [rtile(SXA, k // 2, k % 2, rname, at) for k in range(k0, k0 + nk)]
            r = tiles[0] if nk == 1 else jnp.concatenate(tiles, axis=1)
            if split_last and t == len(TP) - 1:
                p = jnp.concatenate([_dot_nt(lhs[:HM // 2], r), _dot_nt(lhs[HM // 2:], r)], axis=0)
                st['tiles'] += nk
            else:
                p = _dot_nt(lhs, r)
            if k0 == 0:
                TA[t] = p
            else:
                TA[t] += p
        end_dot()

    def t_final_piece(r0, r1):
        def run():
            outs = []
            nr = r1 - r0
            m = lo(nr)
            sgn = jnp.where(m, 1.0, -1.0).astype(F32)

            def ta(rname, op):
                t = TIDX[(rname, op)]
                return jnp.concatenate([TA[t, pl.ds(r + s, 8, stride=2), :]
                                        for r in range(r0, r1, 16) for s in (0, 1)], axis=0)

            def comb(g, ni, na, nb, nc, nd, n11, n22):
                for hf, c, v in ((0, 2 * g, ni + nd - n22 + nb), (1, 2 * g, na + n22),
                                 (0, 2 * g + 1, n11 + nd), (1, 2 * g + 1, ni - n11 + na + nc)):
                    T[c, pl.ds(HM * hf + r0, nr), :] = v
                    outs.append(v)

            comb(0, ta('I1', 'sd'), ta('a1', 'm2'), ta('b1', 'c2'), ta('c1', 'c1'), ta('d1', 'm1'),
                 ta('p11_1', 'o11'), ta('p22_1', 'o22'))
            nb2, nc2 = ta('b2', 'c2'), ta('c2', 'c1')
            q11, q12 = ta('p11_2', 'o11'), ta('p12', 'o12')
            q22, q21 = ta('p22_2', 'o22'), ta('p21', 'o21')
            comb(1, jnp.where(m, ta('E', 'sd'), ta('E', 'sx')), ta('a2', 'm2') * sgn,
                 jnp.where(m, nb2, nc2), jnp.where(m, nc2, nb2), ta('d2', 'm1') * sgn,
                 jnp.where(m, q11, q12), jnp.where(m, q22, q21))
            for hf, (a, b) in enumerate(((q12, q11), (q21, q22))):
                v = a + pltpu.roll(b, 64, 1)
                T[4, pl.ds(HM * hf + r0, nr), :] = v
                outs.append(v)
            return _token(outs)
        return run

    def z_piece():
        zs = jnp.sum(zacc[...], axis=1, keepdims=True)
        zacc[...] = jnp.broadcast_to(zs, (D, 128))
        outs = []
        for d in range(DH):
            t = zacc[pl.ds(d, 32, stride=DH), :]
            zb[pl.ds(32 * d, 32), :] = t
            outs.append(t)
        return _token(outs)

    def a_q(i, at=(), ns=(0, 1)):
        C, mi = sdot(1, SXA, i, at, ns=ns)
        for (hf, b), v in C.items():
            pq[pl.ds(HM * hf, HM), pl.ds(i * BLK + 128 * b, 128)] = _phi(v)
        return mi

    def a_scale(j):
        for n in (0, 1):
            cols = [pl.ds(j * BLK + 128 * b, 128) for b in (n, n + 2)]
            invs = []
            for col in cols:
                den = None
                for d in range(DH):
                    t = pq[pl.ds(32 * d, 32), col] * zb[pl.ds(32 * d, 32), :]
                    den = t if den is None else den + t
                invs.append(1.0 / (den + 1e-6))

            def sc(d, k):
                return pq[pl.ds(32 * d, 32), cols[k]] * invs[k]

            for g in (0, 1):
                for dd in range(4):
                    d1, d2 = 8 * g + dd, 8 * g + dd + 4
                    v = {(d, k): sc(d, k) for d in (d1, d2) for k in (0, 1)}
                    emit_r(scc, j, n, g, 32 * dd, v[(d1, 0)], v[(d1, 1)], v[(d2, 0)], v[(d2, 1)])
                    for d, k in (((d1, 1), (d2, 0)) if g == 1 and dd >= 2 else ((d1, 0), (d2, 1))):
                        scT[pl.ds(16 * d, 16), cols[k]] = _pki(v[(d, k)])
            for d in (16, 17):
                for k in (0, 1):
                    scT[pl.ds(16 * d, 16), cols[k]] = _pki(sc(d, k))

    def a_small_g():
        kvs = []
        for jt, (r0, r1) in enumerate(ROWS):
            n = r1 - r0
            w = 128 if jt < 4 else 64
            tb = jnp.concatenate([T[c, pl.ds(r0, n), :] for c in range(5)], axis=1)[:, :D].astype(BF16)
            g = _dot(tb, wa[:, pl.ds(1152 + 128 * jt, w)])
            rh = (lax.broadcasted_iota(I32, (n, w), 0) + r0) // DH
            ch = (lax.broadcasted_iota(I32, (n, w), 1) + 128 * jt) // DH
            kvs.append(jnp.where(rh == ch, g, 0.0).astype(BF16))
        st['tiles'] += 25
        return kvs

    def a_small_m(buf, kvs):
        for c in range(5):
            wt32[buf, c, pl.ds(0, D), :] = jnp.zeros((D, 128), F32)
        for jt, (r0, r1) in enumerate(ROWS):
            n = r1 - r0
            if jt < 4:
                mrow = _dot(kvs[jt], woa[pl.ds(128 * jt, 128), :])
            else:
                w4 = woa[pl.ds(512, 64), :]
                mrow = jnp.concatenate([
                    _dot(kvs[4], w4[:, :384]),
                    jnp.concatenate([_dot(kvs[4][:48], w4[:, 384:]), _dot(kvs[4][48:], w4[:, 384:])], axis=0)],
                    axis=1)
            for c in range(4):
                wt32[buf, c, pl.ds(r0, n), :] += mrow[:, 128 * c:128 * c + 128]
            wt32[buf, 4, pl.ds(r0, n), pl.ds(0, 64)] += mrow[:, 512:576]
        st['tiles'] += 27

    def b_part(j, p, at=(), cold=False):
        first = j == 0
        lane = lax.broadcasted_iota(I32, (HALO, 128), 1)
        C, mi = sdot(2 + p, SXB, j, at, cold)
        r = {k: _pki(v) for k, v in C.items()}
        for n, d in enumerate(list(range(9, DH)) + list(range(9))):
            hf, dr = divmod(d, 9)
            tl = _upk(jnp.concatenate([r[(hf, b)][16 * dr:16 * dr + 16, :] for b in range(4)], axis=0))
            tt = tl.T.astype(F32)
            att[j, p * DH + d, pl.ds(HALO, 128), :] = tt
            tvals = [tt[120:128, :]]
            if p > 0:
                cur = pltpu.roll(tt[128 - HALO:, :], 32, 1)
                if first:
                    if p == 1:
                        prev = jnp.zeros((HALO, 128), F32)
                    else:
                        prev = jnp.broadcast_to(tt[0:1, :], (HALO, 128))
                else:
                    prev = att[j - 1, p * DH + d, pl.ds(128 + HALO, HALO), :]
                halo = jnp.where(lane < 32, prev, cur)
                att[j, p * DH + d, pl.ds(0, HALO), :] = halo
                tvals.append(halo)
                if j < NB - 1:
                    att[j, p * DH + d, pl.ds(128 + HALO, HALO), :] = cur
            add_due(8 + (n * 20) // DH, _token(tvals))
        return mi

    def att_group(j, g):
        R = ATT_R
        base = HALO + g * R
        ls = [None] * WIN
        csc = None
        for d in range(DH):
            if d % QK_STEP == 0:
                tok = yield
                csc = _or_f32(jnp.full((R, 128), CSC, F32), tok)
            q = att[j, d, pl.ds(base, R), :] * csc
            for w in range(WIN):
                t = q * att[j, DH + d, pl.ds(base - 2 * w, R), :]
                ls[w] = t if ls[w] is None else ls[w] + t
        if g * R < HALO and j == 0:
            pos = (lax.broadcasted_iota(I32, (R, 128), 0) + g * R
                   + (lax.broadcasted_iota(I32, (R, 128), 1) // 32) * 128)
            ls = [ls[0]] + [jnp.where(pos >= 2 * w, ls[w], NEG) for w in range(1, WIN)]
        m = functools.reduce(jnp.maximum, ls)
        es = [jnp.exp2(l - m) for l in ls]
        inv = 1.0 / functools.reduce(lambda a, b: a + b, es)
        ps = None
        for d in range(DH):
            if d % PV_STEP == 0:
                tok = yield
                invt = _or_f32(inv, tok)
                ps = [e * invt for e in es]
            acc = None
            for w in range(WIN):
                t = ps[w] * att[j, 2 * DH + d, pl.ds(base - 2 * w, R), :]
                acc = t if acc is None else acc + t
            att[j, d, pl.ds(base, R), :] = acc

    NPIECE = (128 // ATT_R) * (DH // QK_STEP + DH // PV_STEP)
    state = {'gens': [], 'next': 0, 'ready': 0, 'done': 0}

    def release(mi, n):
        for i in range(n):
            if not state['gens']:
                j = state['next']
                assert j < state['ready']
                state['gens'] = [att_group(j, g) for g in range(128 // ATT_R)]
                for gen in state['gens']:
                    next(gen)
                state['next'] = j + 1
            tok = mark(mi, (i + 0.5) / n)
            gen = state['gens'][0]
            try:
                gen.send(tok)
            except StopIteration:
                state['gens'].pop(0)
            state['done'] += 1

    def ot_piece(j, d1, d2):
        def run():
            assert state['done'] >= NPIECE * (j + 1)
            outs = []
            p1, p2 = [_pk(_upk(_ipk(att[j, d, pl.ds(HALO, 64, stride=2), :],
                                    att[j, d, pl.ds(HALO + 1, 64, stride=2), :])).T)
                      for d in (d1, d2)]

            def put(d, p, b):
                oT[pl.ds(16 * d, 16), pl.ds(j * BLK + 128 * b, 128)] = p[16 * b:16 * b + 16, :]

            if d1 >= 16:
                for b in range(4):
                    put(d1, p1, b)
                    put(d2, p2, b)
                return _token([p1[56:64, :], p2[56:64, :]])
            g, dd = divmod(d1, 8)
            for n in (0, 1):
                s1, s2 = slice(16 * n, 16 * n + 16), slice(16 * n + 32, 16 * n + 48)
                outs += emit_r(oc, j, n, g, 32 * dd, _eo(p1[s1]), _eo(p1[s2]), _eo(p2[s1]), _eo(p2[s2]))
                if g == 1 and dd >= 2:
                    put(d1, p1, n + 2)
                    put(d2, p2, n)
                else:
                    put(d1, p1, n)
                    put(d2, p2, n + 2)
            return _token(outs)
        return run

    def queue_ot(j):
        for d1 in (0, 1, 2, 3, 8, 9, 10, 11):
            queue.append(ot_piece(j, d1, d1 + 4))
        queue.append(ot_piece(j, 16, 17))

    def cat_bf(C):
        return [_upk(jnp.concatenate([_pki(C[(0, b)]), _pki(C[(1, b)])], axis=0)) for b in range(4)]

    def store_t(row0, col0, blk):
        bt = blk.T
        outbuf[pl.ds(row0, 128), pl.ds(col0, blk.shape[0])] = bt
        return _token([bt[112:128, :]])

    def store_part(j, kind, oa, ob, n0, dn):
        for i, b in enumerate((0, 2, 1, 3)):
            rows = []
            if 'a' in kind:
                rows.append(oa[b][0:512])
            if 'm' in kind:
                rows += [oa[b][512:D], ob[b][0:192]]
            if 'b' in kind:
                rows.append(ob[b][192:D])
            col0 = {'a': 0, 'm': 512, 'b': 768}[kind[0]]
            add_due(n0 + dn * i, store_t(j * BLK + 128 * b, col0, jnp.concatenate(rows, axis=0)))

    for name in ('w4', 'x4', 'w0', 'x0', 'w1', 'x1', 'w23', 'x23'):
        in_copy(name).start()

    def wk_t(c):
        wpl[0, :, pl.ds(128 * c, 128)] = _pk(_ktile(wa, c, 512, 640).T[64:, :])

    def kt_part(c0, nc):
        xx = xa[pl.ds(128 * c0, min(128 * nc, D - 128 * c0)), pl.ds(0, BLK)]
        if c0 == 4:
            xx = jnp.concatenate([xx, jnp.zeros_like(xx)], axis=0)
        return _dot(_upk(wpl[0, :, pl.ds(128 * c0, 128 * nc)]), xx)

    def barrier(waits, starts):
        for name in waits:
            in_copy(name).wait()
        for name in starts:
            in_copy(name).start()
        st['tiles'] = 0

    in_copy('w4').wait()
    wk_t(4)
    kT = None
    for c, ws, nxt, tr in [
            (4, ('x4', 'w0'), (), (0,)),
            (0, ('x0', 'w1'), (), (1,)),
            (1, ('x1', 'w23'), ('xa1', 'wa_q'), (2, 3))]:
        barrier(ws, nxt)
        part = kt_part(c, 1)
        for t in tr:
            wk_t(t)
        mk[...] = part[0:8, 0:128]
        kT = part if kT is None else kT + part
    barrier(('x23',), ('xa23', 'wb'))
    for n in (0, 1):
        xc_piece(xa, xca, 0, n, 0)()
    kT = kT + kt_part(2, 2)
    for n in (0, 1):
        xc_piece(xa, xca, 0, n, 1)()
    pk_ops(0, {(hf, b): kT[HM * hf:HM * hf + HM, 128 * b:128 * b + 128] for hf in (0, 1) for b in range(4)})
    for r0 in range(0, HM // 2, 24):
        queue.append(build_piece(0, 0, r0, r0 + 24))
    tdot(0, 2, (10, 14, 18, 22, 26, 30), split_last=True)
    assert not queue

    barrier(('xa1', 'wa_q'), ('wob', 'wa_v', 'woa', 'xb'))
    queue_xc(xa, xca, 1)
    flush()
    queue_prep(3, wa, 0, 640, 0, 1)
    C, _ = sdot(0, SXA, 1, (12, 16, 20, 24, 28, 32), cold=True)
    pk_ops(1, C)
    tdot(2, 1, (3, 6, 9, 12))
    assert not queue
    a_q(0, ns=(0,))

    barrier(('xa23', 'wb'), ())
    queue_xc(xa, xca, 2)
    queue_xc(xa, xca, 3)
    queue_prep(0, wb, 0, 640, 0, 2)
    queue_prep(1, wb, 512, 640, 64, 3)
    queue_prep(2, wb, 1152, 576, 0, 4)
    a_q(0, (6, 10, 14), ns=(1,))
    tdot(3, 1, (1, 5, 9, 13))
    AT8 = (2, 6, 10, 14, 18, 22, 26, 30)
    C, _ = sdot(0, SXA, 2, AT8)
    pk_ops(2, C)
    C, _ = sdot(0, SXA, 3, AT8)
    pk_ops(3, C)
    tdot(4, 2, AT8)
    tdot(6, 2, AT8, split_last=True)
    assert not queue

    barrier(('wob', 'wa_v', 'woa', 'xb'), ())
    queue_xc(xb, xcb, 0)
    flush()
    for r0 in range(0, HM, 96):
        queue.append(t_final_piece(r0, r0 + 96))
    queue.append(z_piece)
    b_part(0, 0, (12, 16, 20, 24, 30), cold=True)
    kvs = a_small_g()
    for c in range(5):
        queue.append(prep_wo_piece(4, c))
    queue_xc(xb, xcb, 1)
    b_part(0, 1, (6, 9, 12, 15, 18, 21, 24, 27, 30))
    a_small_m(0, kvs)
    for r0 in range(0, HM // 2, 48):
        queue.append(build_piece(5, 1, r0, r0 + 48, True))
    for c in range(5):
        queue.append(functools.partial(perm_t_piece, 0, 2, c))
    b_part(0, 2, (8, 11, 14, 17, 20, 23, 26, 29))
    assert not queue
    state['ready'] = 1

    res = {}

    def out_dot(name, m, src, j, at=()):
        C, mi = sdot(m, src, j, at)
        res[name] = cat_bf(C)
        return mi

    def out_block(j):
        out_start(j * BLK, BLK, 0, 2 * D)

    def ready(j):
        state['ready'] = j + 1

    def q_build_m():
        for r0 in range(0, HM // 2, 48):
            queue.append(build_piece(6, 2, r0, r0 + 48, True))

    AT_OT = (8, 11, 14, 17, 20, 23, 26, 29, 32)
    AT4 = (10, 16, 22, 28)
    plan = [
        (lambda: q_build_m(), lambda: b_part(1, 0, AT4)),
        (lambda: queue_xc(xb, xcb, 2), lambda: b_part(1, 1, AT4)),
        (None, lambda: b_part(1, 2)),
        (lambda: (ready(1), a_scale(0)), lambda: b_part(2, 0)),
        (None, lambda: b_part(2, 1)),
        (lambda: queue_ot(0), lambda: b_part(2, 2, AT_OT)),
        (lambda: (ready(2), queue_xc(xb, xcb, 3)), lambda: out_dot('oa0', 6, SSC, 0, AT4)),
        (lambda: store_part(0, 'a', res['oa0'], None, 8, 6), lambda: out_dot('ob0', 5, SO, 0)),
        (lambda: (store_part(0, 'mb', res['oa0'], res['ob0'], 8, 6), out_block(0)), lambda: a_q(1)),
        (lambda: a_scale(1), lambda: b_part(3, 0)),
        (lambda: queue_ot(1), lambda: b_part(3, 1, AT_OT)),
        (None, lambda: b_part(3, 2)),
        (lambda: ready(3), lambda: out_dot('ob1', 5, SO, 1)),
        (lambda: store_part(1, 'b', None, res['ob1'], 8, 6), lambda: out_dot('oa1', 6, SSC, 1)),
        (lambda: (store_part(1, 'am', res['oa1'], res['ob1'], 8, 6), out_block(1), queue_ot(2)),
         lambda: a_q(2, AT_OT)),
        (lambda: a_scale(2), lambda: a_q(3)),
        (None, lambda: out_dot('ob2', 5, SO, 2)),
        (lambda: (store_part(2, 'b', None, res['ob2'], 8, 6), a_scale(3)), lambda: out_dot('oa2', 6, SSC, 2)),
    ]
    for i, (pre, fn) in enumerate(plan):
        if pre is not None:
            pre()
        mi = fn()
        assert not queue
        release(mi, (NB * NPIECE - state['done']) // (len(plan) - i))
    assert state['done'] == NB * NPIECE

    j = NB - 1
    store_part(2, 'am', res['oa2'], res['ob2'], 8, 6)
    out_block(2)
    queue_ot(3)
    out_dot('oa3', 6, SSC, 3, AT_OT)
    oa = res['oa3']
    store_part(j, 'a', oa, None, 4, 3)
    out_start(j * BLK, BLK, 0, 512)
    begin_dot()
    marks = {}
    for n in (0, 1):
        c11, c12, c21, c22 = half(5, SO, j, n, (), marks)
        for i, (b, top, bot) in enumerate(((n + 2, c12, c22), (n, c11, c21))):
            blk = jnp.concatenate([oa[b][512:D], _upk(_pki(top)), _upk(_pki(bot))], axis=0)
            row0 = j * BLK + 128 * b
            if n == 0:
                add_due(24 + 4 * i, store_t(row0, 512, blk))
                out_start(row0, 128, 512, 640)
            else:
                store_t(row0, 512, blk)
                out_start(row0, 128, 512, 640)
    end_dot()
    for cp in outs_started:
        cp.wait()


@jax.jit
def pallas_concat_heads__linear_attn_block__sliding_local_dilated__prompt_kernel(A_x, A_wqkv, A_wo, B_x, B_wqkv, B_wo):
    xa = jnp.transpose(A_x[0])
    xb = jnp.transpose(B_x[0])
    anyspec = pl.BlockSpec(memory_space=pl.ANY)
    comb = pltpu.VMEM((NB, 2, 2, 5, 64, 128), I32)
    out = pl.pallas_call(
        _kernel,
        grid=(1,),
        in_specs=[anyspec] * 6,
        out_specs=anyspec,
        out_shape=jax.ShapeDtypeStruct((S, 2 * D), BF16),
        scratch_shapes=[
            pltpu.VMEM((D, S), BF16),
            pltpu.VMEM((D, S), BF16),
            pltpu.VMEM((D, 3 * D), BF16),
            pltpu.VMEM((D, 3 * D), BF16),
            pltpu.VMEM((D, D), BF16),
            pltpu.VMEM((D, D), BF16),
            pltpu.VMEM((5, 5, KP, 128), F32),
            pltpu.VMEM((3, D // 2, KP), I32),
            pltpu.VMEM((7, HM // 2, 16 * 128), I32),
            comb,
            comb,
            pltpu.VMEM((10, HM // 2, 8 * 128), I32),
            pltpu.VMEM((17, HM, 128), F32),
            pltpu.VMEM((D, S), F32),
            pltpu.VMEM((5, D, 128), F32),
            pltpu.VMEM((D, 128), F32),
            pltpu.VMEM((D, 128), F32),
            pltpu.VMEM((NB, 3 * DH, 128 + 2 * HALO, 128), F32),
            pltpu.VMEM((D // 2, S), I32),
            comb,
            pltpu.VMEM((D // 2, S), I32),
            comb,
            pltpu.VMEM((S, 2 * D), BF16),
            pltpu.VMEM((8, 128), F32),
            pltpu.SemaphoreType.DMA((8,)),
        ],
        compiler_params=pltpu.CompilerParams(
            dimension_semantics=("arbitrary",),
            vmem_limit_bytes=100 * 1024 * 1024),
    )(xa, A_wqkv, A_wo, xb, B_wqkv, B_wo)
    return out.reshape(1, S, 2 * D)
```

```python
import functools
import math

import jax
import jax.numpy as jnp
from jax import lax
import jax.experimental.pallas as pl
import jax.experimental.pallas.tpu as pltpu

S = 2048
D = 576
H = 32
DH = 18
KP = 640
HM = D // 2
BLK = 512
NB = S // BLK
HALO = 16
WIN = 8
ATT_R = 8
QK_STEP = 3
PV_STEP = 6
BAL = 0
EARLYB = 0
LASTF = 0.0
OTL = (7, 10, 13, 16, 19, 22, 25, 28, 31)
FD = 6
FENCE = 'rb pq ao'
TOKW = 4
ATTN = None
DEFER = 0
AT_SC = (4, 7, 10, 13, 16, 19, 22, 25, 28, 31)
SC3 = 17
FDQ = 6
LAZY = 0
TL = (20, 26)
AT_T6 = (2, 4, 6, 8, 10, 13, 16, 19, 22, 25, 28, 31)
AT_B0 = (10, 14, 18, 22, 26, 30, 31)
SC1 = 11
SC2 = 16
ACC = 1
PKR = 48
PK0 = None
PKD = (4, 4)
PKD1 = (1.8, 4)
LB = ('wob', 'wa_v', 'woa', 'xb')
LBN = 0
R4O = 0
ATD = 1
PHI = 1
PL = 1
SC0 = 3
XC3 = 7
FG = 'sx'
RFG = 8
RFO = (16, 8)
RFX = 8
AT_S16 = tuple(range(1, 32, 2))
AT_O18 = (7, 8, 10, 11, 13, 14, 16, 17, 19, 20, 22, 23, 25, 26, 28, 29, 30, 31)
RPH = 8
PHD = ((0, 3), (3, 6), (6, 9), (9, 12), (12, 15), (15, 18))
AT_PH = tuple(range(8, 32))
AT_S8 = (5, 9, 13, 17, 21, 25, 28, 31)
XBS = 1
RS = 0
AT7 = (8, 12, 16, 20, 24, 28, 31)
AT5 = (8, 13, 18, 23, 28)
AT9 = (6, 9, 12, 15, 18, 21, 24, 27, 30)
AQ1 = 0
AT_A1 = (4, 8, 12, 16, 21, 26, 31)
AT_B1 = (6, 9, 12, 15, 18, 21, 24, 27, 30)
AT_B2 = (6, 10, 14, 18, 22, 26, 30)
AT_B3 = (8, 13, 18, 23, 28)
GW = ''
RGO = 12
RGQ = 8
RGB = 8
ATW = None
OT2 = 14
A0 = 26
A1 = 580
RLAG = 16
ADUE = 'qp'
ATQ0 = (3, 6, 9, 12)
AT12 = (2, 6, 10, 14, 18, 22, 26, 30, 34, 38, 42, 46)
F32 = jnp.float32
BF16 = jnp.bfloat16
I32 = jnp.int32
LOG2E = math.log2(math.e)
CSC = (DH ** -0.5) * LOG2E
NEG = -1e9 * LOG2E
ROWS = [(0, 144), (112, 272), (240, 400), (368, 528), (496, 576)]

PASS = ('25', '35', '45', 'G', '12', '32', '42', 'F', '13', '23', '14', '24', '11', '21', '31', '41')
COLD = ('35', '45', '32', '42', '13', '23', '31', '25', 'G', '11', '12', 'F', '21', '41', '14', '24')
PIDX = {p: i for i, p in enumerate(PASS)}
UNITS = {'25': (4, 3), '35': ('s', 3), '45': (4, 's'), 'G': (4, 3), '12': (1, 2), '32': (1, 't'),
         '42': ('t', 2), 'F': (1, 2), '11': (4, 3), '21': (1, 2), '31': (1, 3), '41': (4, 2),
         '13': (1, 3), '23': (1, 3), '14': (4, 2), '24': (4, 2)}
VAR = {(0, 0): 1, (0, 1): 3, (1, 0): 4, (1, 1): 2}
VPOS = {v: k for k, v in VAR.items()}
RAW = {(1, '32'): (0, 1), (1, '12'): (1, 0), (3, '35'): (0, 1), (3, '25'): (1, 0),
       (4, '45'): (0, 1), (2, '42'): (0, 1), (2, '24'): (1, 1)}
USLOT = {}
for _p in PASS:
    for _u in UNITS[_p]:
        USLOT.setdefault(_u if _u in ('s', 't') else (_u, _p), len(USLOT))
NUNIT = len(USLOT)
_H = 0.5
ALPHA = {
    (1, 'F'): ((1, 1, 1), (0, 0, -1)), (1, '32'): ((1, 0, 1), (1, 1, 1)), (1, '21'): ((0, 0, 1),),
    (1, '23'): ((1, 1, 1),), (1, '12'): ((0, 0, 1), (0, 1, 1)), (1, '31'): ((0, 0, 1), (1, 0, 1)),
    (1, '13'): ((0, 1, 1), (1, 1, 1)),
    (3, 'G'): ((0, 0, _H), (0, 1, _H), (1, 1, _H)), (3, '35'): ((0, 0, 1), (0, 1, 1), (1, 0, 1), (1, 1, 1)),
    (3, '11'): ((0, 0, 1),), (3, '13'): ((0, 1, 1), (1, 1, 1)), (3, '25'): ((0, 0, _H), (0, 1, _H)),
    (3, '31'): ((1, 0, 1),), (3, '23'): ((1, 1, _H),),
    (4, 'G'): ((0, 0, _H), (1, 0, -_H), (0, 1, _H), (1, 1, _H)),
    (4, '45'): ((0, 0, _H), (0, 1, _H), (1, 0, _H), (1, 1, _H)), (4, '11'): ((0, 0, 1), (1, 0, -1)),
    (4, '14'): ((0, 1, 1), (1, 1, 1)), (4, '25'): ((0, 0, _H), (0, 1, _H), (1, 0, -_H), (1, 1, -_H)),
    (4, '41'): ((1, 0, 1),), (4, '24'): ((1, 1, 1),),
    (2, 'F'): ((0, 0, _H), (1, 0, -_H), (0, 1, _H), (1, 1, _H)),
    (2, '41'): ((0, 0, _H), (0, 1, _H), (1, 0, _H), (1, 1, _H)), (2, '12'): ((0, 0, _H), (1, 0, -_H)),
    (2, '14'): ((0, 1, _H), (1, 1, _H)), (2, '21'): ((0, 0, _H), (0, 1, _H), (1, 0, -_H), (1, 1, -_H)),
    (2, '42'): ((1, 0, 1),), (2, '24'): ((1, 1, 1),),
}
THIRD = 1.0 / 3.0
ASLOT = {k: i for i, k in enumerate(('e0', 'e1', 'g', 'a0', 'a1', 'b0', 'b1'))}
TORD = ('11', '13', '31', '14', '12', '32', '35', '21', '23', '24', '41', 'F', '25', '42', '45', 'G')


def _r_units(v, b00, b01, b10, b11):
    if v == 1:
        return {'F': b01 + b10, '21': b00 - b10, '23': b11 - b01, '31': b00 + b01, '13': b10 + b11}
    if v == 3:
        p = (b00 - b01) - b01
        r = b00 - b10
        return {'31': p, '11': r, 'G': p - r, '23': (b11 - b10) + b11, '13': b11 - b01}
    d0, d1 = b00 - b01, b10 - b11
    if v == 4:
        return {'25': d1, '11': d0 - d1, '14': b11 - b01, '41': d0 - b01, '24': b11 - d1, 'G': d1 - b01}
    s0 = b00 + b01
    return {'41': s0, '21': d1, 'F': d1 - s0, '12': d0 - d1, '14': (b10 + b11) - s0}


def _c_ops(k00, k01, k10, k11):
    s0, s1 = k00 + k01, k10 + k11
    n0, d1 = k00 - k01, k11 - k10
    f0, f1 = s0 + k00, s1 + k10
    ops = {'11': k00, '13': k01, '14': s0, '12': n0, '31': k10, '32': d1, '35': f1,
           '21': k00 - k10, '25': f0 - f1, '23': k11 - k01, '24': s1 - s0, '41': k00 + k10,
           '42': d1 - n0, '45': f0 + f1, 'F': k10 - k01, 'G': f1 - k01}
    return ops, s0, s1


def _phi(t):
    return jnp.where(t > 0, t + 1.0, jnp.exp(t)) + 1e-6


def _dot(a, b):
    return jnp.dot(a, b, preferred_element_type=F32)


def _dot_nt(a, b):
    return lax.dot_general(a, b, (((1,), (1,)), ((), ())), preferred_element_type=F32)


def _pk(x):
    return pltpu.bitcast(x, I32)


def _upk(x):
    return pltpu.bitcast(x, BF16)


def _pkf(x):
    return _pk(x.astype(BF16))


def _ipk(a, b):
    return pltpu.bitcast(pltpu.pack_elementwise([a, b], packed_dtype=BF16), I32)


def _pki(x):
    out = [_ipk(x[r:r + 8], x[r + 8:r + 16]) for r in range(0, x.shape[0], 16)]
    return out[0] if len(out) == 1 else jnp.concatenate(out, axis=0)


def _par(p, s):
    return pltpu.unpack_elementwise(pltpu.bitcast(p, jnp.uint32), index=s,
                                    packed_dtype=BF16, unpacked_dtype=F32)


class _EO:
    def __init__(self, e, o, p=None):
        self.e, self.o, self.p = e, o, p

    def __add__(self, y):
        return _EO(self.e + y.e, self.o + y.o)

    def __sub__(self, y):
        return _EO(self.e - y.e, self.o - y.o)

    def __mul__(self, c):
        return _EO(self.e * c, self.o * c)

    def sel(self, m, y):
        return _EO(jnp.where(m, self.e, y.e), jnp.where(m, self.o, y.o))

    def pack(self):
        return _ipk(self.e, self.o) if self.p is None else self.p

    def pack_split(self):
        return _pkf(jnp.concatenate([self.e, self.o], axis=0))


def _eo(p):
    return _EO(_par(p, 0), _par(p, 1), p)


def _token(vals):
    accs = []
    n = 0
    for v in vals:
        b = pltpu.bitcast(v, I32)
        for r in range(0, b.shape[0], 8):
            for c in range(0, b.shape[1], 128):
                x = b[r:r + 8, c:c + 128]
                if n < TOKW:
                    accs.append(x)
                else:
                    accs[n % TOKW] = accs[n % TOKW] | x
                n += 1
    while len(accs) > 1:
        accs = [accs[i] | accs[i + 1] if i + 1 < len(accs) else accs[i] for i in range(0, len(accs), 2)]
    acc = accs[0]
    return lax.shift_right_logical(lax.shift_right_logical(acc, 31), 1)


def _or_f32(x, tok):
    if tok is None:
        return x
    return pltpu.bitcast(pltpu.bitcast(x, I32) | tok, F32)


def _off(r, z):
    return r if isinstance(z, int) else pl.multiple_of(r + z, 16)


def _ktile(w_ref, c, col0, ncol, z=0):
    if c < 4:
        return w_ref[pl.ds(_off(128 * c, z), 128), pl.ds(col0, ncol)]
    blk = w_ref[pl.ds(_off(512, z), 64), pl.ds(col0, ncol)]
    return jnp.concatenate([blk, blk], axis=0)


def _kernel(xa_hbm, wa_hbm, woa_hbm, xb_hbm, wb_hbm, wob_hbm, out_hbm,
            xa, xb, wa, wb, woa, wob,
            wt32, wpl, L, xca, xcb, pkc, TA, pq, T, zacc, zb, att, ao, rb, acc, oc, scc, outbuf, mk,
            sem):
    def rows_copy(src, dst, r0, n, col0, ncol, s):
        return pltpu.make_async_copy(src.at[pl.ds(r0, n), pl.ds(col0, ncol)],
                                     dst.at[pl.ds(r0, n), pl.ds(col0, ncol)], sem.at[s])

    def in_copy(name):
        if name == 'w4':
            return rows_copy(wa_hbm, wa, 512, 64, 512, 640, 0)
        if name == 'x4':
            return rows_copy(xa_hbm, xa, 512, 64, 0, BLK, 1)
        if name == 'w0':
            return rows_copy(wa_hbm, wa, 0, 128, 512, 640, 2)
        if name == 'x0':
            return rows_copy(xa_hbm, xa, 0, 128, 0, BLK, 3)
        if name == 'w1':
            return rows_copy(wa_hbm, wa, 128, 128, 512, 640, 4)
        if name == 'x1':
            return rows_copy(xa_hbm, xa, 128, 128, 0, BLK, 5)
        if name == 'w23':
            return rows_copy(wa_hbm, wa, 256, 256, 512, 640, 6)
        if name == 'x23':
            return rows_copy(xa_hbm, xa, 256, 256, 0, BLK, 7)
        if name == 'xa1':
            return rows_copy(xa_hbm, xa, 0, D, BLK, BLK, 0)
        if name == 'wa_q':
            return rows_copy(wa_hbm, wa, 0, D, 0, 512, 1)
        if name == 'xa23':
            return rows_copy(xa_hbm, xa, 0, D, 2 * BLK, 2 * BLK, 2)
        if name == 'wb':
            return pltpu.make_async_copy(wb_hbm, wb, sem.at[3])
        if name == 'wob':
            return pltpu.make_async_copy(wob_hbm, wob, sem.at[4])
        if name == 'wa_v':
            return rows_copy(wa_hbm, wa, 0, D, 1152, 576, 5)
        if name == 'woa':
            return pltpu.make_async_copy(woa_hbm, woa, sem.at[6])
        if name[:2] == 'xb' and len(name) == 3:
            i = int(name[2])
            return rows_copy(xb_hbm, xb, D // XBS * i, D // XBS, 0, S, 7 + i)
        return pltpu.make_async_copy(xb_hbm, xb, sem.at[7])

    outs_started = []

    def out_start(row0, nrow, col0, ncol):
        cp = pltpu.make_async_copy(
            outbuf.at[pl.ds(row0, nrow), pl.ds(col0, ncol)],
            out_hbm.at[pl.ds(row0, nrow), pl.ds(col0, ncol)],
            sem.at[len(outs_started)])
        outs_started.append(cp)
        cp.start()

    lo8 = lax.broadcasted_iota(I32, (8, 128), 1) < 64

    def lo(nr):
        return jnp.concatenate([lo8] * (nr // 8), axis=0)

    queue = []
    due = {}
    later = {}
    gmarks = {}
    plist = []
    state = {'gens': [], 'next': 0, 'ready': 0, 'done': 0}
    st = {'tiles': 0, 'slot': 0, 'gs': 0}

    def fence(kind, ref, idx, vals):
        if kind not in FENCE.split():
            return _token(vals)
        if len(idx) > 2:
            v = ref[(idx[0] + st['dz'],) + tuple(idx[1:-2]) + (pl.ds(idx[-2], 8), pl.ds(idx[-1], 128))]
        else:
            nr = 8 if ref.dtype != BF16 else 16
            v = ref[pl.ds(pl.multiple_of(idx[0] + st['dz'] * nr, nr), nr), pl.ds(idx[1], 128)]
        return _token([v])

    def gate(on, back, x, r0):
        if not on:
            return x
        tok = _token([plist[-back][HM - 8:HM, :]])
        tok = jnp.concatenate([tok] * 5, axis=1)[:, :x.shape[1]]
        p = _pk(x)
        parts = [p[:r0 // 2]] if r0 else []
        return _upk(jnp.concatenate(parts + [p[r0 // 2:r0 // 2 + 8] | tok, p[r0 // 2 + 8:]], axis=0))

    def rel(back):
        pos = (st['tiles'] - back) / 4.0
        r = int(pos)
        row = int((pos - r) * HM) // 8 * 8
        while r not in gmarks:
            r, row = r - 1, HM - 8
        return _token([gmarks[r][row:row + 8, :]])

    def add_due(n, tok):
        due[n] = tok if n not in due else due[n] | tok

    def begin_dot():
        st['slot'] = 0

    def end_dot():
        assert not due, due

    def rtile(src, j, n, name, at):
        orig, comb = src

        def unit(u):
            key = u if u in ('s', 't') else (u, name)
            if orig is not None and key in RAW:
                (g, hi), (k, b) = VPOS[u], RAW[key]
                return _pk(orig[pl.ds(128 * (2 * g + k) + 64 * hi, 64),
                                pl.ds(j * BLK + 128 * (n + 2 * b), 128)])
            return comb[j, n, USLOT[key]]

        s = st['slot']
        if s in at and queue:
            add_due(s, queue.pop(0)())
        for piece in later.pop(st['gs'], ()):
            add_due(s, piece())
        for t in att_emit():
            add_due(s, t)
        st['gs'] += 1
        tok = due.pop(s, None)
        st['slot'] += 1
        st['tiles'] += 1
        p0, p1 = [unit(u) for u in UNITS[name]]
        if tok is not None:
            return _upk(jnp.concatenate([p0[0:8, :] | tok, p0[8:, :], p1], axis=0))
        return _upk(jnp.concatenate([p0, p1], axis=0))

    def half(m, src, j, n, at, marks, cold=False, fin_b=None):
        P = {}
        v = {}
        park = ACC and not cold and m != 0

        def keep(**kw):
            for k, x in kw.items():
                if park:
                    acc[ASLOT[k]] = x
                else:
                    v[k] = x

        def get(k):
            if not park:
                return v[k]
            if 'accdyn' not in st:
                st['accdyn'] = True
                return jnp.concatenate([acc[ASLOT[k] + st['dz'], pl.ds(0, 8), :],
                                        acc[ASLOT[k], pl.ds(8, HM - 8), :]], axis=0)
            return acc[ASLOT[k]]

        def round1():
            keep(e0=P['25'] + P['45'], e1=((P['45'] - P['25']) + P['35']) + P['G'], g=P['G'])

        def round2():
            d0, d1 = (P['42'] - P['12'], P['32'] + P['42']) if park else (v['d0'], v['d1'])
            e0, e1 = get('e0'), get('e1')
            keep(a0=(e0 - d0) + e0, a1=((e1 - d1) + e1) + P['F'],
                 b0=((e0 + d0) - get('g')) - P['F'], b1=e1 + d1)

        def round3():
            s = P['23'] + P['24']
            keep(a0=get('a0') + (P['14'] - P['24']), a1=get('a1') + P['24'])
            v.update(b0=get('b0') + ((P['13'] + P['14']) - s), b1=get('b1') + s)
            if fin_b is not None:
                fin_b(v['b0'], v['b1'])

        steps = [(PASS[:4], round1)] if park else [
            (('25', '45'), lambda: v.update(e0=P['25'] + P['45'], e1=P['45'] - P['25'])),
            (PASS[:4], lambda: v.update(e1=(v['e1'] + P['35']) + P['G'], g=P['G'])),
            (('12', '42', '32'), lambda: v.update(d0=P['42'] - P['12'], d1=P['32'] + P['42']))]
        steps += [(PASS[:8], round2), (PASS[:12], round3)]
        for pat in (COLD if cold else PASS):
            lhs = _upk(L[m, :, pl.ds(128 * PIDX[pat], 128)])
            P[pat] = _dot(lhs, rtile(src, j, n, pat, at))
            marks[(st['tiles'] - 1) // 4] = P[pat]
            gmarks[(st['tiles'] - 1) // 4] = P[pat]
            plist.append(P[pat])
            while steps and all(k in P for k in steps[0][0]):
                steps.pop(0)[1]()
        return [get('a0') + ((P['11'] + P['21']) + P['41']), v['b0'],
                get('a1') + ((P['41'] - P['21']) + P['31']), v['b1']]

    def sdot(m, src, j, at=(), cold=False, ns=(0, 1), fin=None, fd=FD, post=None):
        begin_dot()
        marks = {}
        t0 = st['tiles']
        C = {}
        nslot = 16 * len(ns)
        late = []

        def done(q):
            if fin is not None:
                late.append((st['slot'] + fd, fin(q)))
                if late[-1][0] < nslot:
                    add_due(*late.pop())

        for n in ns:
            c11, c12, c21, c22 = half(m, src, j, n, at, marks, cold and n == ns[0],
                                      lambda b0, b1: done({(0, n + 2): b0, (1, n + 2): b1}))
            C[(0, n)], C[(0, n + 2)], C[(1, n)], C[(1, n + 2)] = c11, c12, c21, c22
            done({(0, n): c11, (1, n): c21})
            if post is not None:
                post(n, (c11, c12, c21, c22))
        end_dot()
        for sl, tok in late:
            add_due(sl - nslot, tok)
        return C, (marks, t0, st['tiles'])

    def mark(mi, f):
        marks, t0, t1 = mi
        pos = (t0 + (t1 - t0) * f) / 4.0
        r = int(pos)
        row = int((pos - r) * HM) // 8 * 8
        return _token([marks[r][row:row + 8, :]])

    def flush():
        while queue:
            queue.pop(0)()

    def emit_l(m, prow, ld, split=False):
        _pkf = _EO.pack_split if split else _EO.pack
        a00, a01, a10, a11 = ld(0, 0), ld(0, 1), ld(1, 0), ld(1, 1)
        nr = a00.e.shape[0]
        m8 = lo(nr)
        c1h = jnp.where(m8, 1.0, 0.5).astype(F32)
        outs = []

        def put(name, v):
            L[m, pl.ds(prow, nr), pl.ds(128 * PIDX[name], 128)] = v
            outs.append(v)

        t1 = a00 + a01
        t4 = a10 + a11
        q2 = t1 * c1h
        q4 = a11 * c1h
        put('13', _pkf(a01 + a11))
        put('23', _pkf(q4))
        put('31', _pkf((a00 + a10).sel(m8, a10)))
        l21_11 = _pkf(a00)
        l12_25 = _pkf(q2)
        l32_35 = _pkf(t4.sel(m8, t4 + t1))
        lf_g = _pkf((q4 - a00).sel(m8, q4 + q2))
        a00, a01, a10, a11 = ld(0, 2), ld(0, 3), ld(1, 2), ld(1, 3)
        e1 = a00 - a10
        s1 = a01 + a11
        put('14', _pkf(s1 * c1h))
        put('24', _pkf(a11))
        h11_12 = _pkf(e1 * c1h)
        h25_21 = _pkf((e1 + (a01 - a11)) * 0.5)
        hg_f = _pkf((e1 + s1) * 0.5)
        hs = _pkf(((a00 + a10) + s1) * 0.5)
        h10 = _pkf(a10)
        put('41', jnp.where(m8, h10, hs))
        put('21', jnp.where(m8, l21_11, h25_21))
        put('11', jnp.where(m8, h11_12, l21_11))
        put('12', jnp.where(m8, l12_25, h11_12))
        put('25', jnp.where(m8, h25_21, l12_25))
        put('F', jnp.where(m8, lf_g, hg_f))
        put('G', jnp.where(m8, hg_f, lf_g))
        r0, r1 = ld(0, 4), ld(1, 4)
        r3 = _pkf((r1 - r0) * THIRD)
        r4 = _pkf(r0 * THIRD)
        put('32', jnp.where(m8, l32_35, r3))
        put('35', jnp.where(m8, r3, l32_35))
        put('42', jnp.where(m8, r4, h10))
        put('45', jnp.where(m8, hs, r4))
        return outs

    def build_piece(m, pb, r0, r1, split=False):
        def run():
            outs = []
            for r in range(r0, r1, 8):
                outs += emit_l(m, r, lambda i, c: _eo(
                    wpl[pb, pl.ds(HM // 2 * i + r, 8), pl.ds(128 * c, 128)]), split=split)
            return fence('L', L, (m, r0, 0), outs)
        return run

    def tr_piece(buf, w_ref, col0, ncol, c):
        def run():
            w = _ktile(w_ref, c, col0, ncol)
            w = gate('q' in GW, RGQ, w, 0) if buf == 3 else gate('b' in GW, RGB, w, 0)
            t = w.T.astype(F32)
            wt32[buf, c, pl.ds(0, ncol), :] = t
            return fence('wt32', wt32, (buf, c, 0, 0), [t[r:r + 8, :] for r in range(120, ncol, 128)] + [t[ncol - 8:, :]])
        return run

    def comb_piece(buf, m, off, d0, d1):
        def run():
            outs = []
            for d in range(d0, d1):
                for hh in (0, 1):
                    outs += emit_l(m, 16 * d + 8 * hh, lambda i, c: _EO(*[
                        wt32[buf, c, pl.ds(off + d + 9 * i + DH * (16 * hh + s), 8, stride=2 * DH), :]
                        for s in (0, 1)]))
            return fence('L', L, (m, 16 * d0, 0), outs)
        return run

    def queue_prep(buf, w_ref, col0, ncol, off, m):
        for c in range(5):
            queue.append(tr_piece(buf, w_ref, col0, ncol, c))
        for d0, d1 in ((0, 2), (2, 4), (4, 6), (6, 8), (8, 9)):
            queue.append(comb_piece(buf, m, off, d0, d1))

    def perm_t_piece(buf, pb, c):
        nrow = 128 if c < 4 else 64
        outs = []
        for kt in range(5):
            ds_ = range(4 * kt, 4 * kt + 4) if kt < 4 else (16, 17, 16, 17)
            rows = [wt32[buf, c, pl.ds(d, 32, stride=DH), :] for d in ds_]
            tile = _pk(_upk(_pki(jnp.concatenate(rows, axis=0))).T[:nrow, :])
            wpl[pb, pl.ds(64 * c, nrow // 2), pl.ds(128 * kt, 128)] = tile
            outs.append(tile)
        return fence('wpl', wpl, (pb, 64 * c, 0), outs)

    def prep_wo_piece(buf, c):
        def run():
            w = gate('o' in GW, RGO, wob[:, pl.ds(128 * c, 128 if c < 4 else 64)], 288).astype(F32)
            if c == 4:
                w = jnp.concatenate([w, jnp.zeros((D, 64), F32)], axis=1)
            wt32[buf, c, pl.ds(0, D), :] = w
            return perm_t_piece(buf, 1, c)
        return run

    def put_unit(comb, j, n, key, r, v):
        v = v.pack() if isinstance(v, _EO) else _pki(v)
        comb[j, n, USLOT[key], pl.ds(r // 2, v.shape[0]), :] = v
        return v

    def emit_r(comb, j, n, g, r, bs, raw):
        var = VAR[(g, r // 64)]
        outs = [put_unit(comb, j, n, (var, p), r % 64, v) for p, v in _r_units(var, *bs).items()]
        if raw:
            for (u, p), (k, b) in RAW.items():
                if u == var:
                    v = put_unit(comb, j, n, (u, p), r % 64, bs[2 * k + b])
                    if not isinstance(bs[0], _EO):
                        outs.append(v)
        return outs

    def emit_rem(comb, j, n, r, b0, b1):
        return [put_unit(comb, j, n, 's', r, b0 + b1), put_unit(comb, j, n, 't', r, (b1 - b0) + b1)]

    def xc_piece(x_ref, comb, j, n, g, rem=None):
        def run():
            outs = []

            def ld(c, b, r):
                return _eo(_pk(x_ref[pl.ds(128 * c + r, 16), pl.ds(j * BLK + 128 * b, 128)]))
            if g == 0 if rem is None else rem:
                for r in range(0, 64, 16):
                    outs += emit_rem(comb, j, n, r, ld(4, n, r), ld(4, n + 2, r))
            for r in range(0, 128, 16):
                outs += emit_r(comb, j, n, g, r, [ld(2 * g + k, n + 2 * b, r)
                                                  for k in (0, 1) for b in (0, 1)], False)
            return fence('comb', comb, (j, n, USLOT[(VAR[(g, 0)], 'F' if g == 0 else 'G')], 0, 0), outs)
        return run

    def xc_fine(x_ref, comb, j, n, g, r0):
        tok = rel(RFX)

        def ld(c, b, r):
            return _eo(_pk(x_ref[pl.ds(128 * c + r, 16), pl.ds(j * BLK + 128 * b, 128)]) | tok)
        outs = []
        for r in range(r0, r0 + 64, 16):
            if g == 2:
                outs += emit_rem(comb, j, n, r, ld(4, n, r), ld(4, n + 2, r))
            else:
                outs += emit_r(comb, j, n, g, r, [ld(2 * g + k, n + 2 * b, r)
                                                  for k in (0, 1) for b in (0, 1)], False)
        return _token(outs)

    def queue_xc(x_ref, comb, j, fine=False):
        if fine and 'x' in FG:
            for n in (0, 1):
                for g, r0 in ((2, 0), (0, 0), (0, 64), (1, 0), (1, 64)):
                    queue.append(functools.partial(xc_fine, x_ref, comb, j, n, g, r0))
            return
        for n in (0, 1):
            for g in (0, 1):
                queue.append(xc_piece(x_ref, comb, j, n, g))

    SXA = (xa, xca)
    SXB = (xb, xcb)
    SO = (None, oc)
    SSC = (None, scc)

    pk_done = set()

    def pk_piece(i, n, quads, r0, r1):
        ops, s0, s1 = _c_ops(*[_phi(q[r0:r1]) for q in quads])
        outs = []
        for name, v in ops.items():
            outs.append(_pki(v))
            pkc[PIDX[name], pl.ds(r0 // 2, (r1 - r0) // 2), pl.ds(128 * (2 * i + n), 128)] = outs[-1]
        for hf, v in enumerate((s0, s1)):
            if i == 0 and n == 0:
                zacc[pl.ds(HM * hf + r0, r1 - r0), :] = v
            else:
                zacc[pl.ds(HM * hf + r0, r1 - r0), :] += v
        pk_done.add((2 * i + n, r0))
        return _token(outs)

    def pk_ops(i, C):
        for n in (0, 1):
            for r0 in range(0, HM, PKR):
                pk_piece(i, n, [C[q] for q in ((0, n), (0, n + 2), (1, n), (1, n + 2))], r0, r0 + PKR)

    def k_dot(i, at, cold=False, sp=PKD):
        def post(n, quads):
            for c, r0 in enumerate(range(0, HM, PKR)):
                later.setdefault(st['gs'] + PK0 + int(sp[n] * c), []).append(
                    functools.partial(pk_piece, i, n, quads, r0, r0 + PKR))
        if PK0 is None:
            pk_ops(i, sdot(0, SXA, i, at, cold)[0])
        else:
            sdot(0, SXA, i, at, cold, post=post)

    def tdot(k0, nk, at=(), pre_fin=None):
        begin_dot()
        late = []
        assert all((k, r) in pk_done for k in range(k0, k0 + nk) for r in range(0, HM, PKR))
        for name in TORD:
            t = PIDX[name]
            lhs = _upk(pkc[t, :, pl.ds(128 * k0, 128 * nk)])
            tiles = [rtile(SXA, k // 2, k % 2, name, at) for k in range(k0, k0 + nk)]
            p = _dot_nt(lhs, tiles[0] if nk == 1 else jnp.concatenate(tiles, axis=1))
            plist.extend([p] * nk)
            gmarks[(st['tiles'] - 1) // 4] = p
            if k0 == 0:
                TA[t] = p
            elif pre_fin is not None and name in TORD[16 - DEFER:]:
                late.append((t, p))
            else:
                TA[t] += p
        end_dot()
        if pre_fin is not None:
            pre_fin()
        for t, p in late:
            TA[t] += p

    def t_final_piece(r0, r1):
        def run():
            outs = []
            c1h = jnp.where(lo8, 1.0, 0.5).astype(F32)
            zero = jnp.zeros((8, 128), F32)

            def sel(a, b):
                return jnp.where(lo8, a, b)

            for r in range(r0, r1, 16):
                for s in (0, 1):
                    ta = {p: TA[PIDX[p], pl.ds(r + s, 8, stride=2), :] for p in PASS}

                    def put(i, c, v):
                        T[c, pl.ds(HM * i + r + 8 * s, 8), :] = v
                        outs.append(v)

                    y3 = sel(ta['32'], ta['35'])
                    y4 = sel(ta['F'], ta['G'])
                    t1 = (sel(ta['12'], ta['25'] + y4)) * c1h + sel(zero, y3)
                    put(0, 0, sel(ta['21'] + (ta['31'] - y4), ta['11']) + t1)
                    put(0, 1, ta['13'] + t1)
                    put(1, 0, ta['31'] + y3)
                    put(1, 1, (ta['13'] + y3) + (ta['23'] + y4) * c1h)
                    hs = sel(ta['45'], ta['41']) * 0.5
                    h10 = sel(ta['41'], ta['42'])
                    g = sel(ta['G'], ta['F']) * 0.5
                    f = sel(ta['25'], ta['21']) * 0.5
                    e1 = sel(ta['11'], ta['12']) * c1h + (f + g)
                    s1 = ta['14'] * c1h + (g + hs)
                    put(0, 2, e1 + hs)
                    put(1, 2, (hs - e1) + h10)
                    put(0, 3, s1 + f)
                    put(1, 3, (s1 - f) + ta['24'])
                    u3 = ta['35'] + pltpu.roll(ta['32'], 64, 1)
                    u4 = ta['42'] + pltpu.roll(ta['45'], 64, 1)
                    put(0, 4, (u4 - u3) * THIRD)
                    put(1, 4, u3 * THIRD)
            return fence('T', T, (0, r0, 0), outs)
        return run

    def z_piece():
        zs = jnp.sum(zacc[...], axis=1, keepdims=True)
        zacc[...] = jnp.broadcast_to(zs, (D, 128))
        outs = []
        for d in range(DH):
            t = zacc[pl.ds(d, 32, stride=DH), :]
            zb[pl.ds(32 * d, 32), :] = t
            outs.append(t)
        return fence('zb', zb, (0, 0), outs)

    def a_q(i, at=(), ns=(0, 1)):
        def fin(C):
            vals = []
            for (hf, b), v in C.items():
                vals.append(v if PHI else _phi(v))
                pq[pl.ds(HM * hf, HM), pl.ds(i * BLK + 128 * b, 128)] = vals[-1]
            return fence('pq', pq, (0, i * BLK + 128 * b), vals)
        return sdot(1, SXA, i, at, ns=ns, fin=fin, fd=FDQ)[1]

    invq = {}

    def a_phi(j):
        dens = {}

        def piece(n, k, d0, d1):
            col = pl.ds(j * BLK + 128 * (n + 2 * k), 128)
            tok = rel(RPH)
            one, l2e = [jnp.concatenate([_or_f32(jnp.full((8, 128), c, F32), tok)] * 4, axis=0)
                        for c in (1.0, LOG2E)]
            den = dens.get((n, k))
            for d in range(d0, d1):
                t = pq[pl.ds(32 * d, 32), col]
                t = jnp.where(t > 0, t + one, jnp.exp2(t * l2e)) + 1e-6
                pq[pl.ds(32 * d, 32), col] = t
                t = t * zb[pl.ds(32 * d, 32), :]
                den = t if den is None else den + t
            dens[(n, k)] = den
            if d1 < DH:
                return _token([den])
            invq[(j, n, k)] = 1.0 / (den + 1e-6)
            return _token([invq[(j, n, k)]])

        for n in (0, 1):
            for k in (0, 1):
                for d0, d1 in PHD:
                    queue.append(functools.partial(piece, n, k, d0, d1))

    def a_scale(j):
        invs = {(n, k): invq[(j, n, k)] for n in (0, 1) for k in (0, 1)} if PHI else {}

        def inv_piece(n):
            for k in (0, 1):
                col = pl.ds(j * BLK + 128 * (n + 2 * k), 128)
                den = None
                for d in range(DH):
                    t = pq[pl.ds(32 * d, 32), col] * zb[pl.ds(32 * d, 32), :]
                    den = t if den is None else den + t
                invs[(n, k)] = 1.0 / (den + 1e-6)
            return _token([invs[(n, 0)], invs[(n, 1)]])

        def sc_piece(n, g, dds, rem):
            inv = [invs[(n, k)] for k in (0, 1)]
            if 's' in FG:
                tok = jnp.concatenate([rel(RFG)] * 4, axis=0)
                inv = [_or_f32(v, tok) for v in inv]

            def sc(d, k):
                return pq[pl.ds(32 * d, 32), pl.ds(j * BLK + 128 * (n + 2 * k), 128)] * inv[k]
            outs = []
            for dd in dds:
                d1, d2 = 8 * g + dd, 8 * g + dd + 4
                outs += emit_r(scc, j, n, g, 32 * dd, [sc(d, k) for d in (d1, d2) for k in (0, 1)], True)
            for d in rem:
                outs += emit_rem(scc, j, n, 32 * (d - 16), sc(d, 0), sc(d, 1))
            var = VAR[(g, dds[0] // 2)]
            return fence('scc', scc, (j, n, USLOT[(var, 'F' if var in (1, 2) else 'G')], 0, 0), outs)

        for n in (0, 1):
            if not PHI:
                queue.append(functools.partial(inv_piece, n))
            for g, dds, rem in ((0, (0, 1), ()), (0, (2, 3), (16,)), (1, (0, 1), (17,)), (1, (2, 3), ())) \
                    if 's' not in FG else [(g, (dd,), {3: (16,), 4: (17,)}.get(4 * g + dd, ()))
                                           for g in (0, 1) for dd in range(4)]:
                queue.append(functools.partial(sc_piece, n, g, dds, rem))

    def a_small_g():
        kvs = []
        for jt, (r0, r1) in enumerate(ROWS):
            n = r1 - r0
            w = 128 if jt < 4 else 64
            tb = jnp.concatenate([T[c, pl.ds(r0, n), :] for c in range(5)], axis=1)[:, :D].astype(BF16)
            wv = wa[:, pl.ds(1152 + 128 * jt, w)]
            if jt < 4 or not BAL:
                g = _dot(tb, wv)
            else:
                g = _dot(tb[:, :512], wv[:512]) + jnp.concatenate(
                    [_dot(tb[a:b, 512:], wv[512:]) for a, b in ((0, 32), (32, 48), (48, 64), (64, 80))], axis=0)
            rh = (lax.broadcasted_iota(I32, (n, w), 0) + r0) // DH
            ch = (lax.broadcasted_iota(I32, (n, w), 1) + 128 * jt) // DH
            kvs.append(jnp.where(rh == ch, g, 0.0).astype(BF16))
        st['tiles'] += 28 if BAL else 25
        return kvs

    def a_small_m(buf, kvs):
        for c in range(5):
            wt32[buf, c, pl.ds(0, D), :] = jnp.zeros((D, 128), F32)
        for jt, (r0, r1) in enumerate(ROWS):
            n = r1 - r0
            if jt < 4:
                mrow = _dot(kvs[jt], woa[pl.ds(128 * jt, 128), :])
            else:
                w4 = woa[pl.ds(512, 64), :]
                if BAL:
                    mrow = jnp.concatenate([
                        _dot(kvs[4], w4[:, :512]),
                        jnp.concatenate([_dot(kvs[4][a:b], w4[:, 512:])
                                         for a, b in ((0, 32), (32, 48), (48, 64), (64, 80))], axis=0)], axis=1)
                else:
                    mrow = jnp.concatenate([
                        _dot(kvs[4], w4[:, :384]),
                        jnp.concatenate([_dot(kvs[4][:48], w4[:, 384:]), _dot(kvs[4][48:], w4[:, 384:])], axis=0)],
                        axis=1)
            for c in range(4):
                wt32[buf, c, pl.ds(r0, n), :] += mrow[:, 128 * c:128 * c + 128]
            wt32[buf, 4, pl.ds(r0, n), pl.ds(0, 64)] += mrow[:, 512:576]
        st['tiles'] += 28 if BAL else 27

    def fin_pack(rs):
        def fin(C):
            vals = []
            for (hf, b), v in C.items():
                vals.append(_pki(v))
                rb[rs, pl.ds(HM // 2 * hf, HM // 2), pl.ds(128 * b, 128)] = vals[-1]
            return fence('rb', rb, (rs, 0, 128 * b), vals)
        return fin

    def b_part(j, p, at=(), cold=False):
        first = j == 0
        lane = lax.broadcasted_iota(I32, (HALO, 128), 1)
        rs = (3 * j + p) % 2
        _, mi = sdot(2 + p, SXB, j, at, cold, fin=fin_pack(rs))
        for n, d in enumerate(list(range(9, DH)) + list(range(9))):
            tl = _upk(jnp.concatenate([rb[rs, pl.ds(16 * d, 16), pl.ds(128 * b, 128)] for b in range(4)], axis=0))
            tt = tl.T.astype(F32)
            att[j, p * DH + d, pl.ds(HALO, 128), :] = tt
            tvals = [tt[120:128, :]]
            if p > 0:
                cur = pltpu.roll(tt[128 - HALO:, :], 32, 1)
                if first:
                    if p == 1:
                        prev = jnp.zeros((HALO, 128), F32)
                    else:
                        prev = jnp.broadcast_to(tt[0:1, :], (HALO, 128))
                else:
                    prev = att[j - 1, p * DH + d, pl.ds(128 + HALO, HALO), :]
                halo = jnp.where(lane < 32, prev, cur)
                att[j, p * DH + d, pl.ds(0, HALO), :] = halo
                tvals.append(halo)
                if j < NB - 1:
                    att[j, p * DH + d, pl.ds(128 + HALO, HALO), :] = cur
            add_due(8 + (n * 20) // DH, fence('att', att, (j, p * DH + d, HALO, 0), tvals))
        return mi

    def att_group(j, g):
        R = ATT_R
        base = HALO + g * R
        ls = [None] * WIN
        csc = None
        for d in range(DH):
            if d % QK_STEP == 0:
                tok = yield
                csc = _or_f32(jnp.full((R, 128), CSC, F32), tok)
            q = att[j, d, pl.ds(base, R), :] * csc
            for w in range(WIN):
                t = q * att[j, DH + d, pl.ds(base - 2 * w, R), :]
                ls[w] = t if ls[w] is None else ls[w] + t
        if g * R < HALO and j == 0:
            pos = (lax.broadcasted_iota(I32, (R, 128), 0) + g * R
                   + (lax.broadcasted_iota(I32, (R, 128), 1) // 32) * 128)
            ls = [ls[0]] + [jnp.where(pos >= 2 * w, ls[w], NEG) for w in range(1, WIN)]
        m = functools.reduce(jnp.maximum, ls)
        es = [jnp.exp2(l - m) for l in ls]
        inv = 1.0 / functools.reduce(lambda a, b: a + b, es)
        ps = None
        fin = _token([inv]) if ATD and 'q' in ADUE else None
        for d in range(DH):
            if d % PV_STEP == 0:
                tok = yield fin
                invt = _or_f32(inv, tok)
                ps = [e * invt for e in es]
                accs = []
            acc = None
            for w in range(WIN):
                t = ps[w] * att[j, 2 * DH + d, pl.ds(base - 2 * w, R), :]
                acc = t if acc is None else acc + t
            ao[j, d, pl.ds(g * R, R), :] = acc
            accs.append(acc)
            fin = None
            if ATD and (d + 1) % PV_STEP == 0 and ('p' in ADUE or ('l' in ADUE and d == DH - 1)):
                fin = fence('ao', ao, (j, d, g * R, 0), accs)
        return fin

    NPIECE = (128 // ATT_R) * (DH // QK_STEP + DH // PV_STEP)

    def att_emit():
        toks = []
        if 'g0' not in state:
            return toks
        tot = NB * NPIECE
        gs = st['gs'] - state['g0']
        if ATW is None:
            n = min(tot, max(0, -(-(gs - A0) * tot // (A1 - A0))))
        else:
            i, sl = divmod(gs, 32)
            lo_, hi_ = (A0, 32) if i == 0 else (0, 32) if i < 18 else (0, A1 - 576)
            n = sum(ATW[:i]) + (0 if i > 18 else min(ATW[i], max(0, -(-(sl + 1 - lo_) * ATW[i] // (hi_ - lo_)))))
            assert sum(ATW) == tot
        n -= state['done']
        for i in range(n):
            if not state['gens']:
                j = state['next']
                assert j < state['ready']
                state['gens'] = [att_group(j, g) for g in range(128 // ATT_R)]
                for gen in state['gens']:
                    next(gen)
                state['next'] = j + 1
            try:
                t = state['gens'][0].send(rel(RLAG - i / n))
            except StopIteration as e:
                t = e.value
                state['gens'].pop(0)
            state['done'] += 1
            if t is not None:
                toks.append(t)
        return toks

    def release(mi, n, f1=1.0):
        for i in range(n):
            if not state['gens']:
                j = state['next']
                assert j < state['ready']
                state['gens'] = [att_group(j, g) for g in range(128 // ATT_R)]
                for gen in state['gens']:
                    next(gen)
                state['next'] = j + 1
            tok = mark(mi, f1 * (i + 0.5) / n)
            gen = state['gens'][0]
            try:
                gen.send(tok)
            except StopIteration:
                state['gens'].pop(0)
            state['done'] += 1

    def ot_piece(j, d1, d2):
        def run():
            assert state['done'] >= NPIECE * (j + 1)
            outs = []
            p1, p2 = [_pk(_upk(_ipk(ao[j, d, pl.ds(0, 64, stride=2), :],
                                    ao[j, d, pl.ds(1, 64, stride=2), :])).T)
                      for d in (d1, d2)]

            for n in (0, 1):
                s1, s2 = slice(16 * n, 16 * n + 16), slice(16 * n + 32, 16 * n + 48)
                bs = [_eo(p1[s1]), _eo(p1[s2]), _eo(p2[s1]), _eo(p2[s2])]
                if d1 >= 16:
                    outs += emit_rem(oc, j, n, 0, bs[0], bs[1]) + emit_rem(oc, j, n, 32, bs[2], bs[3])
                else:
                    g, dd = divmod(d1, 8)
                    outs += emit_r(oc, j, n, g, 32 * dd, bs, True)
            if d1 >= 16:
                return fence('oc', oc, (j, 0, USLOT['s'], 0, 0), outs)
            g, dd = divmod(d1, 8)
            var = VAR[(g, dd // 2)]
            return fence('oc', oc, (j, 0, USLOT[(var, 'F' if var in (1, 2) else 'G')], 16 * (dd % 2), 0), outs)
        return run

    def ot_fine(j, d1, d2):
        ps = []

        def run(n):
            tok = rel(RFO[n])
            if n == 0:
                assert state['done'] >= NPIECE * (j + 1)
                for d in (d1, d2):
                    p = _ipk(ao[j, d, pl.ds(0, 64, stride=2), :], ao[j, d, pl.ds(1, 64, stride=2), :])
                    ps.append(_pk(_upk(jnp.concatenate([p[0:8] | tok, p[8:]], axis=0)).T))
            s1, s2 = slice(16 * n, 16 * n + 16), slice(16 * n + 32, 16 * n + 48)
            bs = [ps[0][s1], ps[0][s2], ps[1][s1], ps[1][s2]]
            if n == 1:
                bs = [b | jnp.concatenate([tok, tok], axis=0) for b in bs]
            bs = [_eo(b) for b in bs]
            if d1 >= 16:
                return _token(emit_rem(oc, j, n, 0, bs[0], bs[1]) + emit_rem(oc, j, n, 32, bs[2], bs[3]))
            g, dd = divmod(d1, 8)
            return _token(emit_r(oc, j, n, g, 32 * dd, bs, True))
        return [functools.partial(run, n) for n in (0, 1)]

    def queue_ot(j):
        if 'o' in FG:
            for d1 in (0, 1, 2, 3, 8, 9, 10, 11):
                queue.extend(ot_fine(j, d1, d1 + 4))
            queue.extend(ot_fine(j, 16, 17))
            return
        for d1 in (0, 1, 2, 3, 8, 9, 10, 11):
            queue.append(ot_piece(j, d1, d1 + 4))
        queue.append(ot_piece(j, 16, 17))

    def cat_bf(C):
        return [_upk(jnp.concatenate([_pki(C[(0, b)]), _pki(C[(1, b)])], axis=0)) for b in range(4)]

    def store_t(row0, col0, blk):
        bt = blk.T
        outbuf[pl.ds(row0, 128), pl.ds(col0, blk.shape[0])] = bt
        return fence('outbuf', outbuf, (row0, col0), [bt[112:128, :]])

    def rbrows(rs, b, r0, r1):
        return _upk(rb[rs, pl.ds(r0 // 2, (r1 - r0) // 2), pl.ds(128 * b, 128)])

    def store_part(j, kind, oa, ob, n0, dn):
        for i, b in enumerate((0, 2, 1, 3)):
            rows = []
            if 'a' in kind:
                rows.append(rbrows(2, b, 0, 512))
            if 'm' in kind:
                rows += [rbrows(2, b, 512, D), rbrows(3, b, 0, 192)]
            if 'b' in kind:
                rows.append(rbrows(3, b, 192, D))
            col0 = {'a': 0, 'm': 512, 'b': 768}[kind[0]]
            add_due(n0 + dn * i, store_t(j * BLK + 128 * b, col0, jnp.concatenate(rows, axis=0)))

    for name in ('w4', 'x4', 'w0', 'x0', 'w1', 'x1', 'w23', 'x23'):
        in_copy(name).start()

    def wk_t(c):
        wpl[0, :, pl.ds(128 * c, 128)] = _pk(_ktile(wa, c, 512, 640).T[64:, :])

    def kt_part(c0, nc):
        xx = xa[pl.ds(128 * c0, min(128 * nc, D - 128 * c0)), pl.ds(0, BLK)]
        if c0 == 4:
            xx = jnp.concatenate([xx, jnp.zeros_like(xx)], axis=0)
        return _dot(_upk(wpl[0, :, pl.ds(128 * c0, 128 * nc)]), xx)

    def barrier(waits, starts):
        if XBS > 1:
            waits, starts = [sum([['xb%d' % i for i in range(XBS)] if n == 'xb' else [n] for n in ns], [])
                             for ns in (waits, starts)]
        for name in waits:
            in_copy(name).wait()
        for name in starts:
            in_copy(name).start()
        st['tiles'] = 0
        gmarks.clear()

    in_copy('w4').wait()
    st['dz'] = jnp.max(_token([_pk(wa[pl.ds(512, 16), pl.ds(512, 128)])]))
    wk_t(4)
    kT = None
    for c, ws, nxt, tr in [
            (4, ('x4', 'w0'), (), (0,)),
            (0, ('x0', 'w1'), (), (1,)),
            (1, ('x1', 'w23'), ('xa1', 'wa_q'), (2, 3))]:
        barrier(ws, nxt)
        part = kt_part(c, 1)
        for t in tr:
            wk_t(t)
        mk[...] = part[0:8, 0:128]
        kT = part if kT is None else kT + part
    barrier(('x23',), ('xa23', 'wb'))
    for n in (0, 1):
        xc_piece(xa, xca, 0, n, 0)()
    kT = kT + kt_part(2, 2)
    for n in (0, 1):
        xc_piece(xa, xca, 0, n, 1)()
    pk_ops(0, {(hf, b): kT[HM * hf:HM * hf + HM, 128 * b:128 * b + 128] for hf in (0, 1) for b in range(4)})
    for r0 in range(0, HM // 2, 24):
        queue.append(build_piece(0, 0, r0, r0 + 24))
    tdot(0, 2, (10, 14, 18, 22, 26, 30))
    assert not queue

    barrier(('xa1', 'wa_q'), LB[:LBN])
    queue_xc(xa, xca, 1)
    flush()
    queue_prep(3, wa, 0, 640, 0, 1)
    k_dot(1, (11, 15, 19, 23, 27, 31), True, PKD1)
    tdot(2, 1, (3, 6, 9, 12))
    assert not queue
    a_q(0, ns=(0,))
    barrier(('xa23', 'wb'), LB[LBN:])
    queue_xc(xa, xca, 2)
    queue_xc(xa, xca, 3)
    queue_prep(0, wb, 0, 640, 0, 2)
    queue_prep(1, wb, 512, 640, 64, 3)
    queue_prep(2, wb, 1152, 576, 0, 4)
    AT8 = (2, 6, 10, 14, 18, 22, 26, 30)
    if RS == 2:
        a_q(0, ATQ0, ns=(1,))
        k_dot(2, AT8)
        k_dot(3, AT8)
        tdot(3, 1, (1, 5, 9, 13))
    elif R4O == 0:
        a_q(0, (6, 10, 14), ns=(1,))
        tdot(3, 1, (1, 5, 9, 13))
        k_dot(2, AT8)
        k_dot(3, AT8)
        tdot(4, 2, AT8)
    else:
        a_q(0, ATQ0, ns=(1,))
        k_dot(2, AT8)
        k_dot(3, AT8)
        tdot(3, 3, AT12)
    if EARLYB:
        barrier(('wob', 'wa_v', 'woa', 'xb'), ())
        queue_xc(xb, xcb, 0)
    if not RS:
        tdot(6, 2, AT_T6 if EARLYB else AT8)
        assert not queue

    def q_wo():
        for c in range(5):
            queue.append(prep_wo_piece(4, c))

    def q_l5():
        for r0 in range(0, HM // 2, 48):
            queue.append(build_piece(5, 1, r0, r0 + 48, True))

    if RS:
        rest = queue[:]
        del queue[:]
        barrier(('wob', 'wa_v', 'woa', 'xb'), ())
        queue_xc(xb, xcb, 0)
        flush()
        queue.extend(rest)
        if RS == 1:
            b_part(0, 0, AT_B0, cold=True)
            assert not queue
            q_wo()
            queue_xc(xb, xcb, 1)
            b_part(0, 1, AT9)
            q_l5()
            b_part(0, 2, (10, 18, 26))
        else:
            b_part(0, 0, AT9, cold=True)
            queue_xc(xb, xcb, 1)
            b_part(0, 1, AT9)
            assert not queue
            q_wo()
            b_part(0, 2, AT5)
    elif AQ1:
        barrier(('wob', 'wa_v', 'woa', 'xb'), ())
        queue_xc(xb, xcb, 0)
        for r0 in range(0, HM, 48):
            queue.append(t_final_piece(r0, r0 + 48))
        queue.append(z_piece)
        for c in range(5):
            queue.append(prep_wo_piece(4, c))
        a_q(1, AT_A1)
        b_part(0, 0, AT_B1)
        assert not queue
        kvs = a_small_g()
        queue_xc(xb, xcb, 1)
        for r0 in range(0, HM // 2, 48):
            queue.append(build_piece(5, 1, r0, r0 + 48, True))
        b_part(0, 1, AT_B2)
        assert not queue
        a_small_m(0, kvs)
        for c in range(5):
            queue.append(functools.partial(perm_t_piece, 0, 2, c))
        b_part(0, 2, AT_B3)
    else:
        if not EARLYB:
            barrier(('wob', 'wa_v', 'woa', 'xb'), ())
            queue_xc(xb, xcb, 0)
            flush()
        for r0 in range(0, HM, 48):
            queue.append(t_final_piece(r0, r0 + 48))
        queue.append(z_piece)
        b_part(0, 0, AT_B0, cold=not EARLYB)
        kvs = a_small_g()
        for c in range(5):
            queue.append(prep_wo_piece(4, c))
        queue_xc(xb, xcb, 1)
        b_part(0, 1, (6, 9, 12, 15, 18, 21, 24, 27, 30))
        a_small_m(0, kvs)
        for r0 in range(0, HM // 2, 48):
            queue.append(build_piece(5, 1, r0, r0 + 48, True))
        for c in range(5):
            queue.append(functools.partial(perm_t_piece, 0, 2, c))
        b_part(0, 2, (8, 11, 14, 17, 20, 23, 26, 29))
    assert not queue
    state['ready'] = 1
    if ATD:
        state['g0'] = st['gs']

    res = {}

    def out_dot(name, m, src, j, at=()):
        res[name] = None
        return sdot(m, src, j, at, fin=fin_pack(2 if name[1] == 'a' else 3))[1]

    def out_block(j):
        out_start(j * BLK, BLK, 0, 2 * D)

    def ready(j):
        state['ready'] = j + 1

    def q_build_m():
        for r0 in range(0, HM // 2, 48):
            queue.append(build_piece(6, 2, r0, r0 + 48, True))

    AT_OT = (7, 10, 13, 16, 19, 22, 25, 28, 31)
    AT4 = (10, 16, 22, 28)
    def q_tfin():
        for r0 in range(0, HM, 48):
            queue.append(t_final_piece(r0, r0 + 48))
        queue.append(z_piece)

    def small_g():
        res['kvs'] = a_small_g()

    def small_m():
        a_small_m(0, res['kvs'])
        for c in range(5):
            queue.append(functools.partial(perm_t_piece, 0, 2, c))

    plan = [
        (lambda: q_build_m(), lambda: b_part(1, 0, AT4)),
        (lambda: queue_xc(xb, xcb, 2), lambda: b_part(1, 1, AT4)),
        (None, lambda: b_part(1, 2)),
        (lambda: (ready(1), a_scale(0)), lambda: b_part(2, 0, AT_SC)),
        (None, lambda: b_part(2, 1)),
    ] if not RS else ([(q_l5, lambda: tdot(4, 2, (10, 18, 26)))] if RS == 2 else []) + [
        (None, lambda: tdot(6, 2)),
        (q_tfin, lambda: b_part(1, 0, AT7)),
        (lambda: (small_g(), queue_xc(xb, xcb, 2)), lambda: b_part(1, 1, AT4)),
        (small_m, lambda: b_part(1, 2, AT5)),
        (lambda: (ready(1), q_build_m()), lambda: b_part(2, 0, AT4)),
        (lambda: a_scale(0), lambda: b_part(2, 1, AT_SC)),
    ]
    plan += [
        (lambda: queue_ot(0), lambda: b_part(2, 2, AT_OT)),
        (lambda: (ready(2), queue_xc(xb, xcb, 3)), lambda: out_dot('oa0', 6, SSC, 0, AT4)),
        (lambda: store_part(0, 'a', res['oa0'], None, 8, 6), lambda: out_dot('ob0', 5, SO, 0)),
        *([(lambda: (store_part(0, 'mb', res['oa0'], res['ob0'], 8, 6), out_block(0)), lambda: b_part(3, 0))]
          if AQ1 else [
            (lambda: (store_part(0, 'mb', res['oa0'], res['ob0'], 8, 6), out_block(0)), lambda: a_q(1)),
            (lambda: a_scale(1) if SC1 == 9 else None, lambda: b_part(3, 0, AT_SC))]),
        (lambda: queue_ot(1), lambda: b_part(3, 1, AT_OT)),
        (lambda: a_scale(1) if SC1 == 11 else None, lambda: b_part(3, 2, AT_SC)),
        (lambda: (ready(3), a_scale(1) if SC1 == 12 else None), lambda: out_dot('ob1', 5, SO, 1, AT_SC)),
        (lambda: (store_part(1, 'b', None, res['ob1'], 8, 6), queue_ot(2) if OT2 == 13 else None),
         lambda: out_dot('oa1', 6, SSC, 1, AT_OT)),
        (lambda: (store_part(1, 'am', res['oa1'], res['ob1'], 8, 6), out_block(1),
                  queue_ot(2) if OT2 == 14 else None),
         lambda: a_q(2, AT_OT)),
        (lambda: a_scale(2) if SC2 == 15 else None, lambda: a_q(3, AT_SC)),
        (lambda: a_scale(2) if SC2 == 16 else None, lambda: out_dot('ob2', 5, SO, 2, AT_SC)),
        (lambda: (store_part(2, 'b', None, res['ob2'], 8, 6), a_scale(3)),
         lambda: out_dot('oa2', 6, SSC, 2, AT_SC)),
    ]
    if PHI:
        AT_S8_ = AT_S16 if 's' in FG else AT_S8
        AT_OT = AT_O18 if 'o' in FG else AT_OT
        AT_X = AT_SC if 'x' in FG else AT4
        plan = [
            (lambda: (q_build_m(), a_phi(0) if PL else None),
             lambda: b_part(1, 0, (5, 6, 7) + AT_PH if PL else AT4)),
            (lambda: queue_xc(xb, xcb, 2, True), lambda: b_part(1, 1, AT_X)),
            (lambda: a_phi(0) if not PL else a_scale(0) if SC0 == 2 else None,
             lambda: b_part(1, 2, AT_S8_ if PL else AT_PH)),
            (lambda: (ready(1), a_scale(0) if SC0 == 3 else None), lambda: b_part(2, 0, AT_S8_)),
            (lambda: a_scale(0) if SC0 == 4 else None, lambda: b_part(2, 1, AT_S8_)),
            (lambda: queue_ot(0), lambda: b_part(2, 2, AT_OT)),
            (lambda: (ready(2), queue_xc(xb, xcb, 3, True) if XC3 == 6 else None),
             lambda: out_dot('oa0', 6, SSC, 0, AT_X)),
            (lambda: (store_part(0, 'a', None, None, 8, 6), queue_xc(xb, xcb, 3, True) if XC3 == 7 else None),
             lambda: out_dot('ob0', 5, SO, 0, AT_X)),
            (lambda: (store_part(0, 'mb', None, None, 8, 6), out_block(0),
                      queue_xc(xb, xcb, 3, True) if XC3 == 8 else None), lambda: a_q(1, AT_X)),
            (lambda: a_phi(1), lambda: b_part(3, 0, AT_PH)),
            (lambda: queue_ot(1), lambda: b_part(3, 1, AT_OT)),
            (lambda: a_scale(1), lambda: b_part(3, 2, AT_S8_)),
            (lambda: ready(3), lambda: a_q(2)),
            (lambda: a_phi(2), lambda: out_dot('ob1', 5, SO, 1, AT_PH)),
            (lambda: (store_part(1, 'b', None, None, 8, 6), queue_ot(2)),
             lambda: out_dot('oa1', 6, SSC, 1, AT_OT)),
            (lambda: (store_part(1, 'am', None, None, 8, 6), out_block(1), a_scale(2)),
             lambda: a_q(3, AT_S8_)),
            (lambda: a_phi(3), lambda: out_dot('ob2', 5, SO, 2, AT_PH)),
            (lambda: (store_part(2, 'b', None, None, 8, 6), a_scale(3)),
             lambda: out_dot('oa2', 6, SSC, 2, AT_S8_)),
        ]
    for i, (pre, fn) in enumerate(plan):
        if pre is not None:
            pre()
        mi = fn()
        assert not queue
        if ATD:
            pass
        elif i == len(plan) - 1:
            release(mi, NB * NPIECE - state['done'], 1.0 + LASTF)
        elif ATTN is not None:
            release(mi, ATTN[i] * NPIECE // 144)
        else:
            release(mi, int((NB * NPIECE - state['done']) // (len(plan) - i + LASTF)))

    j = NB - 1
    store_part(2, 'am', res['oa2'], res['ob2'], 8, 6)
    out_block(2)
    queue_ot(3)
    out_dot('oa3', 6, SSC, 3, AT_O18 if 'o' in FG else OTL)
    oa = res['oa3']
    store_part(j, 'a', oa, None, 4, 3)
    out_start(j * BLK, BLK, 0, 512)
    begin_dot()
    marks = {}

    def fin_last(b, top, bot, slot):
        blk = jnp.concatenate([rbrows(2, b, 512, D), _upk(_pki(top)), _upk(_pki(bot))], axis=0)
        row0 = j * BLK + 128 * b
        tok = store_t(row0, 512, blk)
        if slot is not None:
            add_due(slot, tok)
        out_start(row0, 128, 512, 640)

    for n in (0, 1):
        c11, _, c21, _ = half(5, SO, j, n, (), marks, False,
                              lambda b0, b1: fin_last(n + 2, b0, b1, TL[0] if n == 0 else None))
        fin_last(n, c11, c21, TL[1] if n == 0 else None)
    end_dot()
    for cp in outs_started:
        cp.wait()


@jax.jit
def pallas_concat_heads__linear_attn_block__sliding_local_dilated__prompt_kernel(A_x, A_wqkv, A_wo, B_x, B_wqkv, B_wo):
    xa = jnp.transpose(A_x[0])
    xb = jnp.transpose(B_x[0])
    anyspec = pl.BlockSpec(memory_space=pl.ANY)
    comb = pltpu.VMEM((NB, 2, NUNIT, 32, 128), I32)
    out = pl.pallas_call(
        _kernel,
        grid=(1,),
        in_specs=[anyspec] * 6,
        out_specs=anyspec,
        out_shape=jax.ShapeDtypeStruct((S, 2 * D), BF16),
        scratch_shapes=[
            pltpu.VMEM((D, S), BF16),
            pltpu.VMEM((D, S), BF16),
            pltpu.VMEM((D, 3 * D), BF16),
            pltpu.VMEM((D, 3 * D), BF16),
            pltpu.VMEM((D, D), BF16),
            pltpu.VMEM((D, D), BF16),
            pltpu.VMEM((5, 5, KP, 128), F32),
            pltpu.VMEM((3, D // 2, KP), I32),
            pltpu.VMEM((7, HM // 2, 16 * 128), I32),
            comb,
            comb,
            pltpu.VMEM((16, HM // 2, 8 * 128), I32),
            pltpu.VMEM((16, HM, 128), F32),
            pltpu.VMEM((D, S), F32),
            pltpu.VMEM((5, D, 128), F32),
            pltpu.VMEM((D, 128), F32),
            pltpu.VMEM((D, 128), F32),
            pltpu.VMEM((NB, 3 * DH, 128 + 2 * HALO, 128), F32),
            pltpu.VMEM((NB, DH, 128, 128), F32),
            pltpu.VMEM((4, D // 2, BLK), I32),
            pltpu.VMEM((7, HM, 128), F32),
            comb,
            comb,
            pltpu.VMEM((S, 2 * D), BF16),
            pltpu.VMEM((8, 128), F32),
            pltpu.SemaphoreType.DMA((7 + max(XBS, 1),)),
        ],
        compiler_params=pltpu.CompilerParams(
            dimension_semantics=("arbitrary",),
            vmem_limit_bytes=100 * 1024 * 1024),
    )(xa, A_wqkv, A_wo, xb, B_wqkv, B_wo)
    return out.reshape(1, S, 2 * D)
```
